```python
import jax
import jax.numpy as jnp

def _softmax(x, axis=-1):
    return jax.nn.softmax(x, axis=axis)

def _gelu(x):
    return jax.nn.gelu(x, approximate=True)

def _silu(x):
    return jax.nn.silu(x)

def _sigmoid(x):
    return jax.nn.sigmoid(x)

def _layernorm(x, axis=-1, eps=1e-05):
    m = jnp.mean(x, axis=axis, keepdims=True)
    v = jnp.var(x, axis=axis, keepdims=True)
    return (x - m) / jnp.sqrt(v + eps)

def _scatter_add(tgt, idx, src, axis=0):
    return tgt.at[idx].add(src)

def _segment_sum(src, seg, n):
    return jax.ops.segment_sum(src, seg, n)

class _Rng:

    def __init__(self, key):
        self._k = key

    def _next(self):
        self._k, sub = jax.random.split(self._k)
        return sub

    def normal(self, shape):
        return jax.random.normal(self._next(), shape, dtype=jnp.bfloat16)

    def randint(self, lo, hi, shape):
        return jax.random.randint(self._next(), shape, lo, hi, dtype=jnp.int32)

    def uniform(self, shape, lo=0.0, hi=1.0):
        return jax.random.uniform(self._next(), shape, jnp.bfloat16, lo, hi)

    def permutation(self, n):
        return jax.random.permutation(self._next(), n)
kernel_name = 'adaLN_cond__sliding_block_cached__dense_activation_mish__decode'

def setup_inputs():
    _rng = _Rng(jax.random.key(int.from_bytes(__import__("os").urandom(4), "little")))
    _w = lambda a: (lambda t: t.astype(jnp.bfloat16) if jnp.issubdtype(t.dtype, jnp.floating) else t)(jnp.asarray(a))

    def _A_setup():
        B, Sq, D = (1, 1, 640)
        Hq, Hkv, Sk, Dh = (32, 32, 32768, 192)
        assert Hq % Hkv == 0, (Hq, Hkv)
        return {'x': _w((lambda *s: _rng.normal(s) * 0.05)(B, Sq, D)), 'k_cache': _w((lambda *s: _rng.normal(s) * 0.05)(B, Hkv, Sk, Dh)), 'v_cache': _w((lambda *s: _rng.normal(s) * 0.05)(B, Hkv, Sk, Dh)), 'wq': _w((lambda *s: _rng.normal(s) * 0.05)(D, Hq * Dh) * D ** (-0.5)), 'wo': _w((lambda *s: _rng.normal(s) * 0.05)(Hq * Dh, D) * (Hq * Dh) ** (-0.5))}
    _A_in = _A_setup()

    def _B_setup():
        B, S, D, F = (1, 1, 640, 1536)
        return {'x': _w((lambda *s: _rng.normal(s) * 0.05)(B, S, D)), 'w1': _w((lambda *s: _rng.normal(s) * 0.05)(D, F) * D ** (-0.5)), 'b1': _w((lambda *s: _rng.normal(s) * 0.05)(F)), 'w2': _w((lambda *s: _rng.normal(s) * 0.05)(F, D) * F ** (-0.5))}
    _B_in = _B_setup()
    return {'A_x': _A_in['x'], 'A_k_cache': _A_in['k_cache'], 'A_v_cache': _A_in['v_cache'], 'A_wq': _A_in['wq'], 'A_wo': _A_in['wo'], 'B_x': _B_in['x'], 'B_w1': _B_in['w1'], 'B_b1': _B_in['b1'], 'B_w2': _B_in['w2'], 'c': _w((lambda *s: _rng.normal(s) * 0.05)(1, 640)), 'w_mod': _w((lambda *s: _rng.normal(s) * 0.05)(640, 6 * 640) * 640 ** (-0.5))}

def reference(A_x, A_k_cache, A_v_cache, A_wq, A_wo, B_x, B_w1, B_b1, B_w2, c, w_mod):

    def _A_ref(x, k_cache, v_cache, wq, wo):
        B, Sq, D = x.shape
        Hq, Dh = (32, 192)
        Hkv, Sk = (k_cache.shape[1], k_cache.shape[2])
        W = min(4096, max(256, Sk // 4))
        rep = Hq // Hkv
        q = (lambda x, *d: x.transpose(*d))((x @ wq).reshape(B, Sq, Hq, Dh), 0, 2, 1, 3)
        k = jnp.repeat(k_cache[:, :, Sk - W:, :], rep, axis=1)
        v = jnp.repeat(v_cache[:, :, Sk - W:, :], rep, axis=1)
        scores = jnp.einsum('bhqd,bhkd->bhqk', q, k) * Dh ** (-0.5)
        p = _softmax(scores, axis=-1)
        o = jnp.einsum('bhqk,bhkd->bhqd', p, v)
        return (lambda x, *d: x.transpose(*d))(o, 0, 2, 1, 3).reshape(B, Sq, Hq * Dh) @ wo

    def _B_ref(x, w1, b1, w2):
        h = jnp.einsum('bsd,df->bsf', x, w1) + b1
        sp = jnp.log1p(jnp.exp(-jnp.abs(h))) + jnp.where(h > 0, h, jnp.zeros_like(h))
        act = h * jnp.tanh(sp)
        return jnp.einsum('bsf,fd->bsd', act, w2)
    x = A_x
    mod = (_silu(c) @ w_mod).reshape(c.shape[0], 6, 1, -1)
    sa, ca, ga, sb, cb, gb = (mod[:, 0].copy(), mod[:, 1].copy(), mod[:, 2].copy(), mod[:, 3].copy(), mod[:, 4].copy(), mod[:, 5].copy())
    h = _layernorm(x, axis=-1) * (1 + ca) + sa
    x = x + ga * _A_ref(h, A_k_cache, A_v_cache, A_wq, A_wo)
    h = _layernorm(x, axis=-1) * (1 + cb) + sb
    x = x + gb * _B_ref(h, B_w1, B_b1, B_w2)
    return x
```

```python
import jax
import jax.numpy as jnp
from jax import lax
from jax.experimental import pallas as pl
from jax.experimental.pallas import tpu as pltpu

D = 640
HQ = 32
DH = 192
F = 1536
EPS = 1e-5
f32 = jnp.float32
bf16 = jnp.bfloat16

G = 2
NB = 3
WO_CH = 8
W1_CH = 5
W2_CH = 4
GB_CH = 5
R = G * DH
NG = HQ // G


def _rowchunks(n, ch):
    return [(i * (n // ch), n // ch) for i in range(ch)]


def _kernel(x_hbm, c_hbm, b1_hbm, wmod_hbm, wq_hbm, k_hbm, v_hbm, wo_hbm, w1_hbm, w2_hbm,
            o_ref,
            x_v, c_v, b1_v, wmodA_v, wgb_v, wq_v, kbuf, vbuf, wo_v, w1_v, w2_v, q_s, o_s,
            sem_small, sem_a, sem_k, sem_v, sem_wo, sem_w1, sem_w2, sem_gb):
    SK = k_hbm.shape[1]
    W = kbuf.shape[2]
    w0 = SK - W

    cp_c = pltpu.make_async_copy(c_hbm, c_v, sem_small.at[0])
    cp_x = pltpu.make_async_copy(x_hbm, x_v, sem_small.at[1])
    cp_b1 = pltpu.make_async_copy(b1_hbm, b1_v, sem_small.at[2])
    cp_wmodA = pltpu.make_async_copy(wmod_hbm.at[:, pl.ds(0, 5 * D)], wmodA_v, sem_a.at[0])
    cp_wq = pltpu.make_async_copy(wq_hbm, wq_v, sem_a.at[1])

    def kcopy(g, slot):
        return pltpu.make_async_copy(k_hbm.at[pl.ds(g * R, R), pl.ds(w0, W)], kbuf.at[slot], sem_k.at[slot])

    def vcopy(g, slot):
        return pltpu.make_async_copy(v_hbm.at[pl.ds(g * R, R), pl.ds(w0, W)], vbuf.at[slot], sem_v.at[slot])

    wo_cp = [pltpu.make_async_copy(wo_hbm.at[pl.ds(s, n), :], wo_v.at[pl.ds(s, n), :], sem_wo.at[i])
             for i, (s, n) in enumerate(_rowchunks(HQ * DH, WO_CH))]
    w1_cp = [pltpu.make_async_copy(w1_hbm.at[pl.ds(s, n), :], w1_v.at[pl.ds(s, n), :], sem_w1.at[i])
             for i, (s, n) in enumerate(_rowchunks(D, W1_CH))]
    w2_cp = [pltpu.make_async_copy(w2_hbm.at[pl.ds(s, n), :], w2_v.at[pl.ds(s, n), :], sem_w2.at[i])
             for i, (s, n) in enumerate(_rowchunks(F, W2_CH))]
    gb_cp = [pltpu.make_async_copy(wmod_hbm.at[pl.ds(s, n), pl.ds(5 * D, D)], wgb_v.at[pl.ds(s, n), :], sem_gb.at[i])
             for i, (s, n) in enumerate(_rowchunks(D, GB_CH))]

    cp_c.start()
    cp_x.start()
    cp_wmodA.start()
    cp_wq.start()
    cp_b1.start()
    for g in range(NB):
        kcopy(g, g).start()
        vcopy(g, g).start()

    cp_c.wait()
    cp_x.wait()
    c = c_v[...].astype(f32)
    sc = (c * jax.nn.sigmoid(c)).astype(bf16)
    x = x_v[...].astype(f32)

    def ln(z):
        m = jnp.mean(z, axis=-1, keepdims=True)
        zc = z - m
        v = jnp.mean(zc * zc, axis=-1, keepdims=True)
        return zc * lax.rsqrt(v + EPS)

    xn = ln(x)
    cp_wmodA.wait()
    modA = jnp.dot(sc, wmodA_v[...], preferred_element_type=f32)
    sa = modA[:, 0:D]
    ca = modA[:, D:2 * D]
    ga = modA[:, 2 * D:3 * D]
    sb = modA[:, 3 * D:4 * D]
    cb = modA[:, 4 * D:5 * D]
    h = (xn * (1.0 + ca) + sa).astype(bf16)
    cp_wq.wait()
    q = jnp.dot(h, wq_v[...], preferred_element_type=f32)
    q_s[...] = q * (DH ** -0.5)

    row = lax.broadcasted_iota(jnp.int32, (8, R), 0)
    col = lax.broadcasted_iota(jnp.int32, (8, R), 1)
    diag = (col >= row * DH) & (col < (row + 1) * DH)

    def group(g, carry):
        slot = g % NB
        off = pl.multiple_of(g * R, 128)
        qg = q_s[:, pl.ds(off, R)]
        qbd = jnp.where(diag, jnp.broadcast_to(qg, (8, R)), 0.0).astype(bf16)
        kcopy(g, slot).wait()
        s = jnp.dot(qbd, kbuf[slot], preferred_element_type=f32)

        @pl.when(g + NB < NG)
        def _():
            kcopy(g + NB, slot).start()

        m = jnp.max(s, axis=-1, keepdims=True)
        p = jnp.exp(s - m)
        l = jnp.sum(p, axis=-1, keepdims=True)
        vcopy(g, slot).wait()
        ov = lax.dot_general(p.astype(bf16), vbuf[slot], (((1,), (1,)), ((), ())),
                             preferred_element_type=f32)

        @pl.when(g + NB < NG)
        def _():
            vcopy(g + NB, slot).start()

        @pl.when(g + NB == NG)
        def _():
            for cp in wo_cp + w1_cp + w2_cp + gb_cp:
                cp.start()

        ov = jnp.where(diag, ov / l, 0.0)
        o_s[:, pl.ds(off, R)] = jnp.sum(ov, axis=0, keepdims=True)
        return carry

    lax.fori_loop(0, NG, group, 0)

    acc = jnp.zeros((1, D), f32)
    for i, (s, n) in enumerate(_rowchunks(HQ * DH, WO_CH)):
        wo_cp[i].wait()
        acc = acc + jnp.dot(o_s[:, s:s + n].astype(bf16), wo_v[s:s + n, :], preferred_element_type=f32)
    x1 = x + ga * acc
    h2 = (ln(x1) * (1.0 + cb) + sb).astype(bf16)
    cp_b1.wait()
    b1 = b1_v[...].astype(f32)
    hh = jnp.concatenate([b1[j:j + 1, :] for j in range(F // 128)], axis=1)
    for i, (s, n) in enumerate(_rowchunks(D, W1_CH)):
        w1_cp[i].wait()
        hh = hh + jnp.dot(h2[:, s:s + n], w1_v[s:s + n, :], preferred_element_type=f32)
    sp = jnp.log1p(jnp.exp(-jnp.abs(hh))) + jnp.maximum(hh, 0.0)
    act = (hh * jnp.tanh(sp)).astype(bf16)
    y = jnp.zeros((1, D), f32)
    for i, (s, n) in enumerate(_rowchunks(F, W2_CH)):
        w2_cp[i].wait()
        y = y + jnp.dot(act[:, s:s + n], w2_v[s:s + n, :], preferred_element_type=f32)
    gb = jnp.zeros((1, D), f32)
    for i, (s, n) in enumerate(_rowchunks(D, GB_CH)):
        gb_cp[i].wait()
        gb = gb + jnp.dot(sc[:, s:s + n], wgb_v[s:s + n, :], preferred_element_type=f32)
    o_ref[...] = (x1 + gb * y).astype(o_ref.dtype)


@jax.jit
def pallas_adaLN_cond__sliding_block_cached__dense_activation_mish__decode_kernel(
    A_x: jax.Array,
    A_k_cache: jax.Array,
    A_v_cache: jax.Array,
    A_wq: jax.Array,
    A_wo: jax.Array,
    B_x: jax.Array,
    B_w1: jax.Array,
    B_b1: jax.Array,
    B_w2: jax.Array,
    c: jax.Array,
    w_mod: jax.Array,
):
    B, H, SK, dh = A_k_cache.shape
    W = min(4096, max(256, SK // 4))
    kt = jnp.swapaxes(A_k_cache, 2, 3).reshape(H * dh, SK)
    vt = jnp.swapaxes(A_v_cache, 2, 3).reshape(H * dh, SK)
    x2 = A_x.reshape(1, D)
    b1 = B_b1.reshape(F // 128, 128)
    out = pl.pallas_call(
        _kernel,
        out_shape=jax.ShapeDtypeStruct((1, D), A_x.dtype),
        in_specs=[pl.BlockSpec(memory_space=pl.ANY)] * 10,
        out_specs=pl.BlockSpec(memory_space=pltpu.VMEM),
        scratch_shapes=[
            pltpu.VMEM((1, D), bf16), pltpu.VMEM((1, D), bf16), pltpu.VMEM((F // 128, 128), bf16),
            pltpu.VMEM((D, 5 * D), bf16), pltpu.VMEM((D, D), bf16), pltpu.VMEM((D, HQ * DH), bf16),
            pltpu.VMEM((NB, R, W), bf16), pltpu.VMEM((NB, R, W), bf16),
            pltpu.VMEM((HQ * DH, D), bf16), pltpu.VMEM((D, F), bf16), pltpu.VMEM((F, D), bf16),
            pltpu.VMEM((1, HQ * DH), f32), pltpu.VMEM((1, HQ * DH), f32),
            pltpu.SemaphoreType.DMA((3,)), pltpu.SemaphoreType.DMA((2,)),
            pltpu.SemaphoreType.DMA((NB,)), pltpu.SemaphoreType.DMA((NB,)),
            pltpu.SemaphoreType.DMA((WO_CH,)), pltpu.SemaphoreType.DMA((W1_CH,)),
            pltpu.SemaphoreType.DMA((W2_CH,)), pltpu.SemaphoreType.DMA((GB_CH,)),
        ],
        compiler_params=pltpu.CompilerParams(vmem_limit_bytes=100 * 1024 * 1024),
    )(x2, c, b1, w_mod, A_wq, kt, vt, A_wo, B_w1, B_w2)
    return out.reshape(A_x.shape)
```

```python
import functools
import jax
import jax.numpy as jnp
from jax import lax
from jax.experimental import pallas as pl
from jax.experimental.pallas import tpu as pltpu

D = 640
HQ = 32
DH = 192
F = 1536
EPS = 1e-5
f32 = jnp.float32
bf16 = jnp.bfloat16
G = 2
R = G * DH
NG = HQ // G


def make(kv_piece=(8, 2048), kv_order='cr', pat=(0, 1, 1), NCH=8, wpat=(0, 1, 1),
         wmod_piece=(8, 1920), wq_piece=(8, 2048), wo_piece=(16, 640), w1_piece=(8, 1536), w2_piece=(16, 640),
         w_order='cr', w2_split=(768, 512, 128, 128), compute=True, nobc=True):

    S_C, S_X, S_B1, S_WMOD, S_WQ, S_K, S_V, S_WO, S_W1, S_W2 = 0, 1, 2, 3, 4, 5, 7, 9, 12, 13
    NSEM = S_W2 + len(w2_split)

    def issue(src, dst, sem, row0, col0, nrows, ncols, piece, order, pattern, ch, nch, drow0=0, dcol0=0):
        pr, pc = piece
        nr, nc = nrows // pr, ncols // pc
        assert nr * pr == nrows and nc * pc == ncols
        npieces = nr * nc
        ppc = npieces // nch
        assert ppc * nch == npieces, (npieces, nch)
        inner = nr if order == 'cr' else nc
        if ppc % inner == 0:
            base_o = ch * (ppc // inner)
            oi = [(base_o + k // inner, k % inner) for k in range(ppc)]
        elif inner % ppc == 0:
            per = inner // ppc
            o = ch // per
            b = (ch % per) * ppc
            oi = [(o, b + k) for k in range(ppc)]
        else:
            oi = [((ch * ppc + k) // inner, (ch * ppc + k) % inner) for k in range(ppc)]
        for k, (o, i) in enumerate(oi):
            c, r = (o, i) if order == 'cr' else (i, o)
            ro = r * pr
            co = c * pc
            sr = row0 + ro
            dr = drow0 + ro
            sc_ = col0 + co
            dc = dcol0 + co
            if not isinstance(sr, int): sr = pl.multiple_of(sr, 8)
            if not isinstance(dr, int): dr = pl.multiple_of(dr, 8)
            if not isinstance(sc_, int): sc_ = pl.multiple_of(sc_, 128)
            if not isinstance(dc, int): dc = pl.multiple_of(dc, 128)
            pltpu.make_async_copy(src.at[pl.ds(sr, pr), pl.ds(sc_, pc)], dst.at[pl.ds(dr, pr), pl.ds(dc, pc)], sem
                                  ).start(priority=pattern[k % len(pattern)])

    def wait_all(buf, sem):
        pltpu.make_async_copy(buf, buf, sem).wait()

    def kernel(*refs):
        pl.run_scoped(functools.partial(body, *refs), pltpu.SemaphoreType.DMA((NSEM,)))

    def body(x_hbm, c_hbm, b1_hbm, wmod_hbm, wq_hbm, k_hbm, v_hbm, wo_hbm, w1_hbm, w2_hbm,
             o_ref,
             x_v, c_v, b1_v, wmod_v, wq_v, kbuf, vbuf, wo_v, w1_v, w2_v, mod_s, q_s, o_s, s_s, p_s,
             sems):
        SK = k_hbm.shape[1]
        W = kbuf.shape[2]
        w0 = SK - W
        CW = W // NCH

        def issue_k(g, ch, nch):
            slot = g % 2
            issue(k_hbm, kbuf.at[slot], sems.at[S_K + slot], g * R, w0, R, W, kv_piece, kv_order, pat, ch, nch)

        def issue_v(g, ch, nch):
            slot = g % 2
            issue(v_hbm, vbuf.at[slot], sems.at[S_V + slot], g * R, w0, R, W, kv_piece, kv_order, pat, ch, nch)

        WOP = HQ * DH // 3

        def issue_wo(part, ch, nch):
            issue(wo_hbm, wo_v, sems.at[S_WO + part], part * WOP, 0, WOP, D, wo_piece, 'cr', wpat, ch, nch,
                  drow0=part * WOP)

        def loop(n, fn, init=0):
            return lax.fori_loop(0, n, fn, init)

        cp_c = pltpu.make_async_copy(c_hbm, c_v, sems.at[S_C])
        cp_x = pltpu.make_async_copy(x_hbm, x_v, sems.at[S_X])
        cp_b1 = pltpu.make_async_copy(b1_hbm, b1_v, sems.at[S_B1])

        def _wmod(ch, cr):
            issue(wmod_hbm, wmod_v, sems.at[S_WMOD], 0, 0, D, 6 * D, wmod_piece, w_order, wpat, ch, 10)
            return cr
        _wmod(0, 0)
        cp_c.start()
        cp_x.start()
        cp_b1.start()
        lax.fori_loop(1, 10, _wmod, 0)

        def _wq(ch, cr):
            issue(wq_hbm, wq_v, sems.at[S_WQ], 0, 0, D, HQ * DH, wq_piece, w_order, wpat, ch, 15 if w_order == 'cr' and False else (10 if w_order == 'rc' else 15))
            return cr
        loop(10 if w_order == 'rc' else 15, _wq)

        cp_c.wait()
        cp_x.wait()
        c = c_v[...].astype(f32)
        sc = (c * jax.nn.sigmoid(c)).astype(bf16)
        x = x_v[...].astype(f32)

        def ln(z):
            m = jnp.mean(z, axis=-1, keepdims=True)
            zc = z - m
            v = jnp.mean(zc * zc, axis=-1, keepdims=True)
            return zc * lax.rsqrt(v + EPS)

        xn = ln(x)
        wait_all(wmod_v, sems.at[S_WMOD])

        def _mod(ch, cr):
            issue_k(0, ch, 6)
            off = pl.multiple_of(ch * D, 128)
            mod_s[:, pl.ds(off, D)] = jnp.dot(sc, wmod_v[:, pl.ds(off, D)], preferred_element_type=f32)
            return cr
        loop(6, _mod)

        h = (xn * (1.0 + mod_s[:, D:2 * D]) + mod_s[:, 0:D]).astype(bf16)

        def _v0(ch, cr):
            issue_v(0, ch, NCH)
            return cr
        loop(NCH, _v0)
        wait_all(wq_v, sems.at[S_WQ])

        QC = HQ * DH // 8

        def _q(ch, cr):
            issue_k(1, ch, 8)
            off = pl.multiple_of(ch * QC, 128)
            q_s[:, pl.ds(off, QC)] = jnp.dot(h, wq_v[:, pl.ds(off, QC)], preferred_element_type=f32) * (DH ** -0.5)
            return cr
        loop(8, _q)

        row = lax.broadcasted_iota(jnp.int32, (8, R), 0)
        col = lax.broadcasted_iota(jnp.int32, (8, R), 1)
        diag = (col >= row * DH) & (col < (row + 1) * DH)

        def group(g, issue_a, issue_b):
            slot = g % 2
            off = g * R if isinstance(g, int) else pl.multiple_of(g * R, 128)
            qg = q_s[:, pl.ds(off, R)]
            qbd = jnp.where(diag, jnp.broadcast_to(qg, (8, R)), 0.0).astype(bf16)
            wait_all(kbuf.at[slot], sems.at[S_K + slot])

            def qk(ch, cr):
                issue_a(ch)
                co = pl.multiple_of(ch * CW, 128)
                if compute:
                    s_s[:, pl.ds(co, CW)] = jnp.dot(qbd, kbuf[slot, :, pl.ds(co, CW)], preferred_element_type=f32)
                else:
                    s_s[:, pl.ds(co, CW)] = kbuf[slot, 0:8, pl.ds(co, CW)].astype(f32)
                return cr
            loop(NCH, qk)

            s = s_s[...]
            m = jnp.max(s, axis=-1, keepdims=True)
            p = jnp.exp(s - m)
            l = jnp.sum(p, axis=-1, keepdims=True)
            p_s[...] = p
            wait_all(vbuf.at[slot], sems.at[S_V + slot])

            def pv(ch, acc):
                issue_b(ch)
                co = pl.multiple_of(ch * CW, 128)
                if compute:
                    return acc + lax.dot_general(p_s[:, pl.ds(co, CW)].astype(bf16), vbuf[slot, :, pl.ds(co, CW)],
                                                 (((1,), (1,)), ((), ())), preferred_element_type=f32)
                else:
                    return acc + vbuf[slot, 0:8, pl.ds(co, R)].astype(f32)
            ov = loop(NCH, pv, jnp.zeros((8, R), f32))
            ov = jnp.where(diag, ov / l, 0.0)
            o_s[:, pl.ds(off, R)] = jnp.sum(ov, axis=0, keepdims=True)

        def main(g, cr):
            group(g, lambda ch: issue_v(g + 1, ch, NCH), lambda ch: issue_k(g + 2, ch, NCH))
            return cr
        loop(NG - 2, main)
        group(NG - 2, lambda ch: issue_v(NG - 1, ch, NCH), lambda ch: issue_wo(0, ch, NCH))
        group(NG - 1, lambda ch: issue_wo(1, ch, NCH), lambda ch: issue_wo(2, ch, NCH))

        WC = WOP // 8

        def wo_part(part, issue_fn, acc):
            wait_all(wo_v.at[pl.ds(part * WOP, WOP), :], sems.at[S_WO + part])

            def it(ch, a):
                issue_fn(ch)
                ro = pl.multiple_of(part * WOP + ch * WC, 128)
                return a + jnp.dot(o_s[:, pl.ds(ro, WC)].astype(bf16), wo_v[pl.ds(ro, WC), :],
                                   preferred_element_type=f32)
            return loop(8, it, acc)

        acc = jnp.zeros((1, D), f32)
        acc = wo_part(0, lambda ch: issue(w1_hbm, w1_v, sems.at[S_W1], 0, 0, D, F, w1_piece, 'cr', wpat, ch, 8), acc)

        w2_starts = [sum(w2_split[:i]) for i in range(len(w2_split))]

        def issue_w2_first(ch):
            issue(w2_hbm, w2_v, sems.at[S_W2], 0, 0, w2_split[0], D, w2_piece, 'cr', wpat, ch, 8)
        acc = wo_part(1, issue_w2_first, acc)
        for i in range(1, len(w2_split)):
            issue(w2_hbm, w2_v, sems.at[S_W2 + i], w2_starts[i], 0, w2_split[i], D, w2_piece, 'cr', wpat, 0, 1,
                  drow0=w2_starts[i])
        wait_all(wo_v.at[pl.ds(2 * WOP, WOP), :], sems.at[S_WO + 2])
        acc = acc + jnp.dot(o_s[:, 2 * WOP:].astype(bf16), wo_v[2 * WOP:, :], preferred_element_type=f32)

        x1 = x + mod_s[:, 2 * D:3 * D] * acc
        h2 = (ln(x1) * (1.0 + mod_s[:, 4 * D:5 * D]) + mod_s[:, 3 * D:4 * D]).astype(bf16)
        cp_b1.wait()
        b1 = b1_v[...].astype(f32)
        hh = jnp.concatenate([b1[j:j + 1, :] for j in range(F // 128)], axis=1)
        wait_all(w1_v, sems.at[S_W1])
        hh = hh + jnp.dot(h2, w1_v[...], preferred_element_type=f32)
        sp = jnp.log1p(jnp.exp(-jnp.abs(hh))) + jnp.maximum(hh, 0.0)
        act = (hh * jnp.tanh(sp)).astype(bf16)
        gb = mod_s[:, 5 * D:6 * D]
        y = jnp.zeros((1, D), f32)
        for i, n in enumerate(w2_split):
            s0 = w2_starts[i]
            wait_all(w2_v.at[pl.ds(s0, n), :], sems.at[S_W2 + i])
            y = y + jnp.dot(act[:, s0:s0 + n], w2_v[s0:s0 + n, :], preferred_element_type=f32)
        o_ref[...] = (x1 + gb * y).astype(o_ref.dtype)

    @jax.jit
    def f(A_x, A_k_cache, A_v_cache, A_wq, A_wo, B_x, B_w1, B_b1, B_w2, c, w_mod):
        B, H, SK, dh = A_k_cache.shape
        W = min(4096, max(256, SK // 4))
        kt = jnp.swapaxes(A_k_cache, 2, 3).reshape(H * dh, SK)
        vt = jnp.swapaxes(A_v_cache, 2, 3).reshape(H * dh, SK)
        x2 = A_x.reshape(1, D)
        b1 = B_b1.reshape(F // 128, 128)
        out = pl.pallas_call(
            kernel,
            out_shape=jax.ShapeDtypeStruct((1, D), A_x.dtype),
            in_specs=[pl.BlockSpec(memory_space=pl.ANY)] * 10,
            out_specs=pl.BlockSpec(memory_space=pltpu.VMEM),
            scratch_shapes=[
                pltpu.VMEM((1, D), bf16), pltpu.VMEM((1, D), bf16), pltpu.VMEM((F // 128, 128), bf16),
                pltpu.VMEM((D, 6 * D), bf16), pltpu.VMEM((D, HQ * DH), bf16),
                pltpu.VMEM((2, R, W), bf16), pltpu.VMEM((2, R, W), bf16),
                pltpu.VMEM((HQ * DH, D), bf16), pltpu.VMEM((D, F), bf16), pltpu.VMEM((F, D), bf16),
                pltpu.VMEM((1, 6 * D), f32), pltpu.VMEM((1, HQ * DH), f32), pltpu.VMEM((1, HQ * DH), f32),
                pltpu.VMEM((8, W), f32), pltpu.VMEM((8, W), f32),
            ],
            compiler_params=pltpu.CompilerParams(vmem_limit_bytes=100 * 1024 * 1024, disable_bounds_checks=nobc),
        )(x2, c, b1, w_mod, A_wq, kt, vt, A_wo, B_w1, B_w2)
        return out.reshape(A_x.shape)
    return f


_impl = make(**dict(kv_piece=(128,128)))


@jax.jit
def pallas_adaLN_cond__sliding_block_cached__dense_activation_mish__decode_kernel(
    A_x: jax.Array,
    A_k_cache: jax.Array,
    A_v_cache: jax.Array,
    A_wq: jax.Array,
    A_wo: jax.Array,
    B_x: jax.Array,
    B_w1: jax.Array,
    B_b1: jax.Array,
    B_w2: jax.Array,
    c: jax.Array,
    w_mod: jax.Array,
):
    return _impl(A_x, A_k_cache, A_v_cache, A_wq, A_wo, B_x, B_w1, B_b1, B_w2, c, w_mod)
```

```python
import functools
import jax
import jax.numpy as jnp
from jax import lax
from jax.experimental import pallas as pl
from jax.experimental.pallas import tpu as pltpu

D = 640
HQ = 32
DH = 192
F = 1536
EPS = 1e-5
f32 = jnp.float32
bf16 = jnp.bfloat16
G = 2
R = G * DH
NG = HQ // G


def _mo(v, m):
    return v if isinstance(v, int) else pl.multiple_of(v, m)


def _flat_order(n, st):
    ns = (n + st - 1) // st
    return [m * st + t for t in range(st) for m in range(ns) if m * st + t < n]


def make(split=((8, 0), (88, 1), (8, 0), (88, 1)), NCH=8, wpat=(0, 1, 1, 1, 1, 1), wq_pc=1024, wmod_st=51, wo_st=51,
         wo_tpc=3, w1_pc=512, compute=True, wcompute=True, nobc=True, tpat=(0, 1, 1, 1)):

    HR = sum(r for r, _ in split)
    assert R % HR == 0
    NH = R // HR
    S_C, S_X, S_B1, S_WMOD, S_WQ, S_K, S_V, S_WO, S_W1, S_W2 = 0, 1, 2, 3, 4, 5, 7, 9, 10, 11
    NSEM = S_W2 + 3

    def issue_kv(src, dst, sem, row0, col0, W, ch, nch):
        nct = W // 128
        tot = NH * nct
        per = tot // nch
        assert per * nch == tot
        if nct % per == 0:
            cph = nct // per
            hc = [(ch // cph, (ch % cph) * per + k) for k in range(per)]
        else:
            hc = [((ch * per + k) // nct, (ch * per + k) % nct) for k in range(per)]
        for (hf, c) in hc:
            o = 0
            for (r, p) in split:
                pltpu.make_async_copy(
                    src.at[pl.ds(_mo(row0 + hf * HR + o, 8), r), pl.ds(_mo(col0 + c * 128, 128), 128)],
                    dst.at[pl.ds(_mo(hf * HR + o, 8), r), pl.ds(_mo(c * 128, 128), 128)], sem,
                ).start(priority=p)
                o += r

    def issue_flat(src, dst, sem, pc, nc, idx, pattern, k0=0):
        for k, j in enumerate(idx):
            rt, c = j // nc, j % nc
            pltpu.make_async_copy(src.at[pl.ds(rt * 8, 8), pl.ds(c * pc, pc)],
                                  dst.at[pl.ds(rt * 8, 8), pl.ds(c * pc, pc)], sem,
                                  ).start(priority=pattern[(k0 + k) % len(pattern)])

    def issue_streams(streams, rt0, nrt, pattern):
        k = 0
        ncmax = max(s[6] for s in streams)
        for i in range(nrt):
            for c in range(ncmax):
                for (src, dst, sem, sr0, dr0, pc, nc) in streams:
                    if c >= nc:
                        continue
                    ro = (rt0 + i) * 8
                    pltpu.make_async_copy(
                        src.at[pl.ds(_mo(sr0 + ro, 8), 8), pl.ds(c * pc, pc)],
                        dst.at[pl.ds(_mo(dr0 + ro, 8), 8), pl.ds(c * pc, pc)], sem,
                    ).start(priority=pattern[k % len(pattern)])
                    k += 1

    def wait_all(buf, sem):
        pltpu.make_async_copy(buf, buf, sem).wait()

    def kernel(*refs):
        pl.run_scoped(functools.partial(body, *refs), pltpu.SemaphoreType.DMA((NSEM,)))

    def body(x_hbm, c_hbm, b1_hbm, wmod_hbm, wq_hbm, k_hbm, v_hbm, wo_hbm, w1_hbm, w2_hbm,
             o_ref,
             x_v, c_v, b1_v, wmod_v, wq_v, kbuf, vbuf, wo_v, w1_v, w2a_v, w2b_v, w2c_v,
             mod_s, q_s, o_s, s_s, p_s, hh_s, y_s,
             sems):
        SK = k_hbm.shape[1]
        W = kbuf.shape[2]
        w0 = SK - W
        CW = W // NCH

        def issue_k(g, ch, nch):
            slot = g % 2
            issue_kv(k_hbm, kbuf.at[slot], sems.at[S_K + slot], g * R, w0, W, ch, nch)

        def issue_v(g, ch, nch):
            slot = g % 2
            issue_kv(v_hbm, vbuf.at[slot], sems.at[S_V + slot], g * R, w0, W, ch, nch)

        def loop(n, fn, init=0):
            return lax.fori_loop(0, n, fn, init)

        NWO = HQ * DH // 8
        wo_ns = NWO // wo_st
        wo_streams = [(wo_hbm, wo_v, sems.at[S_WO], 8 * wo_st * m, 8 * wo_st * m, D, 1) for m in range(wo_ns)]

        cp_c = pltpu.make_async_copy(c_hbm, c_v, sems.at[S_C])
        cp_x = pltpu.make_async_copy(x_hbm, x_v, sems.at[S_X])
        cp_b1 = pltpu.make_async_copy(b1_hbm, b1_v, sems.at[S_B1])

        wmod_idx = _flat_order(80 * 6, wmod_st)
        wq_nc = HQ * DH // wq_pc
        wq_idx = _flat_order(80 * wq_nc, 256 * 128 // wq_pc)
        issue_flat(wmod_hbm, wmod_v, sems.at[S_WMOD], D, 6, wmod_idx[:30], wpat)
        cp_c.start()
        cp_x.start()
        cp_b1.start()
        issue_flat(wmod_hbm, wmod_v, sems.at[S_WMOD], D, 6, wmod_idx[30:], wpat)
        issue_flat(wq_hbm, wq_v, sems.at[S_WQ], wq_pc, wq_nc, wq_idx[:96], wpat)

        cp_c.wait()
        cp_x.wait()
        c = c_v[...].astype(f32)
        sc = (c * jax.nn.sigmoid(c)).astype(bf16)
        x = x_v[...].astype(f32)

        def ln(z):
            m = jnp.mean(z, axis=-1, keepdims=True)
            zc = z - m
            v = jnp.mean(zc * zc, axis=-1, keepdims=True)
            return zc * lax.rsqrt(v + EPS)

        y_s[0:1, :] = ln(x)
        issue_flat(wq_hbm, wq_v, sems.at[S_WQ], wq_pc, wq_nc, wq_idx[96:], wpat)
        wait_all(wmod_v, sems.at[S_WMOD])

        def _mod(ch, cr):
            issue_k(0, ch, 8)
            off = pl.multiple_of(jnp.minimum(ch, 5) * D, 128)
            if wcompute:
                mod_s[:, pl.ds(off, D)] = jnp.dot(sc, wmod_v[:, pl.ds(off, D)], preferred_element_type=f32)
            else:
                mod_s[:, pl.ds(off, D)] = wmod_v[0:1, pl.ds(off, D)].astype(f32)
            return cr
        loop(6, _mod)
        issue_k(0, 6, 8)
        issue_k(0, 7, 8)

        h = (y_s[0:1, :] * (1.0 + mod_s[:, D:2 * D]) + mod_s[:, 0:D]).astype(bf16)
        wait_all(wq_v, sems.at[S_WQ])

        QC = HQ * DH // 8

        def _q(ch, cr):
            issue_v(0, ch, 8)
            off = pl.multiple_of(ch * QC, 128)
            if wcompute:
                q_s[:, pl.ds(off, QC)] = jnp.dot(h, wq_v[:, pl.ds(off, QC)], preferred_element_type=f32) * (DH ** -0.5)
            else:
                q_s[:, pl.ds(off, QC)] = wq_v[0:1, pl.ds(off, QC)].astype(f32)
            return cr
        loop(8, _q)

        row = lax.broadcasted_iota(jnp.int32, (8, R), 0)
        col = lax.broadcasted_iota(jnp.int32, (8, R), 1)
        diag = (col >= row * DH) & (col < (row + 1) * DH)

        def group(g, issue_a, issue_b):
            slot = g % 2
            off = _mo(g * R, 128)
            qg = q_s[:, pl.ds(off, R)]
            qbd = jnp.where(diag, jnp.broadcast_to(qg, (8, R)), 0.0).astype(bf16)
            wait_all(kbuf.at[slot], sems.at[S_K + slot])

            def qk(ch, cr):
                issue_a(ch)
                co = pl.multiple_of(ch * CW, 128)
                if compute:
                    s_s[:, pl.ds(co, CW)] = jnp.dot(qbd, kbuf[slot, :, pl.ds(co, CW)], preferred_element_type=f32)
                else:
                    s_s[:, pl.ds(co, CW)] = kbuf[slot, 0:8, pl.ds(co, CW)].astype(f32)
                return cr
            loop(NCH, qk)

            s = s_s[...]
            m = jnp.max(s, axis=-1, keepdims=True)
            p = jnp.exp(s - m)
            l = jnp.sum(p, axis=-1, keepdims=True)
            p_s[...] = p
            wait_all(vbuf.at[slot], sems.at[S_V + slot])

            def pv(ch, acc):
                issue_b(ch)
                co = pl.multiple_of(ch * CW, 128)
                if compute:
                    return acc + lax.dot_general(p_s[:, pl.ds(co, CW)].astype(bf16), vbuf[slot, :, pl.ds(co, CW)],
                                                 (((1,), (1,)), ((), ())), preferred_element_type=f32)
                else:
                    return acc + vbuf[slot, 0:8, pl.ds(0, R)].astype(f32)
            ov = loop(NCH, pv, jnp.zeros((8, R), f32))
            ov = jnp.where(diag, ov / l, 0.0)
            o_s[:, pl.ds(off, R)] = jnp.sum(ov, axis=0, keepdims=True)

        def main(g, cr):
            group(g, lambda ch: issue_k(g + 1, ch, NCH), lambda ch: issue_v(g + 1, ch, NCH))
            return cr
        loop(NG - 1, main)
        group(NG - 1, lambda ch: issue_streams(wo_streams, ch * wo_tpc, wo_tpc, wpat),
              lambda ch: issue_streams(wo_streams, (NCH + ch) * wo_tpc, wo_tpc, wpat))

        w1_nc = F // w1_pc
        w1_str = [(w1_hbm, w1_v, sems.at[S_W1], 160 * m, 160 * m, w1_pc, w1_nc) for m in range(4)]
        w2a_str = [(w2_hbm, w2a_v, sems.at[S_W2], 384 * m, 256 * m, D, 1) for m in range(4)]
        w2b_str = [(w2_hbm, w2b_v, sems.at[S_W2 + 1], 384 * m + 256, 128 * m, D, 1) for m in range(3)]
        w2c_str = [(w2_hbm, w2c_v, sems.at[S_W2 + 2], 384 * 3 + 256, 0, D, 1)]

        issue_streams(wo_streams, 2 * NCH * wo_tpc, wo_st - 2 * NCH * wo_tpc, wpat)
        issue_flat(wo_hbm, wo_v, sems.at[S_WO], D, 1, list(range(wo_ns * wo_st, NWO)), wpat)
        issue_streams(w1_str, 0, 8, tpat)
        wait_all(wo_v, sems.at[S_WO])

        def wo_dot(m):
            lo = _mo(768 * m, 128)
            if wcompute:
                return jnp.dot(o_s[:, pl.ds(lo, 768)].astype(bf16), wo_v[pl.ds(lo, 768), :], preferred_element_type=f32)
            return wo_v[pl.ds(lo, 16), :][0:1].astype(f32) + o_s[:, pl.ds(lo, 128)][:, 0:1]

        def wo_a(ch, a):
            issue_streams(w1_str, 8 + 2 * ch, 2, tpat)
            return a + wo_dot(ch)
        acc = loop(6, wo_a, jnp.zeros((1, D), f32))

        def wo_b(ch, a):
            issue_streams(w2a_str, 6 * ch, 6, tpat)
            return a + wo_dot(6 + ch)
        acc = loop(2, wo_b, acc)

        x1 = x + mod_s[:, 2 * D:3 * D] * acc
        h2 = (ln(x1) * (1.0 + mod_s[:, 4 * D:5 * D]) + mod_s[:, 3 * D:4 * D]).astype(bf16)
        y_s[0:1, :] = h2.astype(f32)
        y_s[1:2, :] = x1
        issue_streams(w2a_str, 12, 4, tpat)
        cp_b1.wait()
        b1 = b1_v[...].astype(f32)
        hh_s[...] = jnp.concatenate([b1[j:j + 1, :] for j in range(F // 128)], axis=1)
        wait_all(w1_v, sems.at[S_W1])

        def w1_it(ch, cr):
            issue_streams(w2a_str, 16 + 4 * ch, 4, tpat)
            co = pl.multiple_of(ch * 384, 128)
            if wcompute:
                hh = hh_s[:, pl.ds(co, 384)] + jnp.dot(y_s[0:1, :].astype(bf16), w1_v[:, pl.ds(co, 384)],
                                                       preferred_element_type=f32)
            else:
                hh = hh_s[:, pl.ds(co, 384)] + w1_v[0:1, pl.ds(co, 384)].astype(f32)
            sp = jnp.log1p(jnp.exp(-jnp.abs(hh))) + jnp.maximum(hh, 0.0)
            hh_s[:, pl.ds(co, 384)] = hh * jnp.tanh(sp)
            return cr
        loop(4, w1_it)

        issue_streams(w2b_str, 0, 16, tpat)
        issue_streams(w2c_str, 0, 16, tpat)

        def dotw(a, wv):
            if wcompute:
                return jnp.dot(a.astype(bf16), wv[...], preferred_element_type=f32)
            return wv[0:1, :].astype(f32) + a[:, 0:1]

        wait_all(w2a_v, sems.at[S_W2])
        act_a = jnp.concatenate([hh_s[:, 384 * m:384 * m + 256] for m in range(4)], axis=1)
        y_s[2:3, :] = dotw(act_a, w2a_v)
        wait_all(w2b_v, sems.at[S_W2 + 1])
        act_b = jnp.concatenate([hh_s[:, 384 * m + 256:384 * m + 384] for m in range(3)], axis=1)
        gb = mod_s[:, 5 * D:6 * D]
        y_s[3:4, :] = y_s[1:2, :] + gb * (y_s[2:3, :] + dotw(act_b, w2b_v))
        wait_all(w2c_v, sems.at[S_W2 + 2])
        o_ref[...] = (y_s[3:4, :] + gb * dotw(hh_s[:, 384 * 3 + 256:], w2c_v)).astype(o_ref.dtype)

    @jax.jit
    def f(A_x, A_k_cache, A_v_cache, A_wq, A_wo, B_x, B_w1, B_b1, B_w2, c, w_mod):
        B, H, SK, dh = A_k_cache.shape
        W = min(4096, max(256, SK // 4))
        kt = jnp.swapaxes(A_k_cache, 2, 3).reshape(H * dh, SK)
        vt = jnp.swapaxes(A_v_cache, 2, 3).reshape(H * dh, SK)
        x2 = A_x.reshape(1, D)
        b1 = B_b1.reshape(F // 128, 128)
        out = pl.pallas_call(
            kernel,
            out_shape=jax.ShapeDtypeStruct((1, D), A_x.dtype),
            in_specs=[pl.BlockSpec(memory_space=pl.ANY)] * 10,
            out_specs=pl.BlockSpec(memory_space=pltpu.VMEM),
            scratch_shapes=[
                pltpu.VMEM((1, D), bf16), pltpu.VMEM((1, D), bf16), pltpu.VMEM((F // 128, 128), bf16),
                pltpu.VMEM((D, 6 * D), bf16), pltpu.VMEM((D, HQ * DH), bf16),
                pltpu.VMEM((2, R, W), bf16), pltpu.VMEM((2, R, W), bf16),
                pltpu.VMEM((HQ * DH, D), bf16), pltpu.VMEM((D, F), bf16),
                pltpu.VMEM((1024, D), bf16), pltpu.VMEM((384, D), bf16), pltpu.VMEM((128, D), bf16),
                pltpu.VMEM((1, 6 * D), f32), pltpu.VMEM((1, HQ * DH), f32), pltpu.VMEM((1, HQ * DH), f32),
                pltpu.VMEM((8, W), f32), pltpu.VMEM((8, W), f32), pltpu.VMEM((1, F), f32), pltpu.VMEM((8, D), f32),
            ],
            compiler_params=pltpu.CompilerParams(vmem_limit_bytes=100 * 1024 * 1024, disable_bounds_checks=nobc),
        )(x2, c, b1, w_mod, A_wq, kt, vt, A_wo, B_w1, B_w2)
        return out.reshape(A_x.shape)
    return f


_impl = make(**dict())


@jax.jit
def pallas_adaLN_cond__sliding_block_cached__dense_activation_mish__decode_kernel(
    A_x: jax.Array,
    A_k_cache: jax.Array,
    A_v_cache: jax.Array,
    A_wq: jax.Array,
    A_wo: jax.Array,
    B_x: jax.Array,
    B_w1: jax.Array,
    B_b1: jax.Array,
    B_w2: jax.Array,
    c: jax.Array,
    w_mod: jax.Array,
):
    return _impl(A_x, A_k_cache, A_v_cache, A_wq, A_wo, B_x, B_w1, B_b1, B_w2, c, w_mod)
```

```python
import functools
import jax
import jax.numpy as jnp
from jax import lax
from jax.experimental import pallas as pl
from jax.experimental.pallas import tpu as pltpu

D = 640
HQ = 32
DH = 192
F = 1536
EPS = 1e-5
f32 = jnp.float32
bf16 = jnp.bfloat16
G = 2
R = G * DH
NG = HQ // G


def _mo(v, m):
    return v if isinstance(v, int) else pl.multiple_of(v, m)


def _flat_order(n, st):
    ns = (n + st - 1) // st
    return [m * st + t for t in range(st) for m in range(ns) if m * st + t < n]


def make(split=((32, 0),) + ((32, 1),) * 5, NCH=8, wpat=(0, 1, 1, 1, 1, 1), wq_pc=1024, wmod_pc=640, wmod_st=51, wo_st=51,
         wo_tpc=3, w1_pc=512, compute=True, wcompute=True, nobc=True, tpat=(0, 1, 1, 1), ppat=(0, 1, 1, 1, 1, 1),
         pro_loop=False, vpu_end=True, c1=96):

    HR = sum(r for r, _ in split)
    assert R % HR == 0
    NH = R // HR
    S_C, S_X, S_B1, S_WMOD, S_WQ, S_K, S_V, S_WO, S_W1, S_W2 = 0, 1, 2, 3, 4, 5, 7, 9, 10, 11
    NSEM = S_W2 + 4

    def issue_kv(src, dst, sem, row0, col0, W, ch, nch):
        nct = W // 128
        tot = NH * nct
        per = tot // nch
        assert per * nch == tot
        if nct % per == 0:
            cph = nct // per
            hc = [(ch // cph, (ch % cph) * per + k) for k in range(per)]
        else:
            hc = [((ch * per + k) // nct, (ch * per + k) % nct) for k in range(per)]
        for (hf, c) in hc:
            o = 0
            for (r, p) in split:
                pltpu.make_async_copy(
                    src.at[pl.ds(_mo(row0 + hf * HR + o, 8), r), pl.ds(_mo(col0 + c * 128, 128), 128)],
                    dst.at[pl.ds(_mo(hf * HR + o, 8), r), pl.ds(_mo(c * 128, 128), 128)], sem,
                ).start(priority=p)
                o += r

    def issue_flat(src, dst, sem, pc, nc, idx, pattern, k0=0):
        for k, j in enumerate(idx):
            rt, c = j // nc, j % nc
            pltpu.make_async_copy(src.at[pl.ds(rt * 8, 8), pl.ds(c * pc, pc)],
                                  dst.at[pl.ds(rt * 8, 8), pl.ds(c * pc, pc)], sem,
                                  ).start(priority=pattern[(k0 + k) % len(pattern)])

    def issue_flat_loop(src, dst, sem, pc, nc, n, st, pattern, after_first=None):
        ns_full = n // st
        rem = n - ns_full * st

        def step(u, ks, ms):
            i = 0
            for k in ks:
                for m in ms(k):
                    j0 = st * m + k
                    ro = _mo((j0 // nc + u) * 8, 8)
                    co = (j0 % nc) * pc
                    pltpu.make_async_copy(src.at[pl.ds(ro, 8), pl.ds(co, pc)], dst.at[pl.ds(ro, 8), pl.ds(co, pc)], sem,
                                          ).start(priority=pattern[i % len(pattern)])
                    i += 1

        nu = st // nc
        nu_p = rem // nc
        u0 = 0
        if after_first is not None:
            step(0, range(nc), lambda k: range(ns_full + (1 if k < rem else 0)))
            after_first()
            u0 = 1
        if nu_p > u0:
            lax.fori_loop(u0, nu_p, lambda u, c: (step(u, range(nc), lambda k: range(ns_full + 1)), c)[1], 0)
            u0 = nu_p
        if rem and u0 == nu_p and nu_p < nu and (rem % nc):
            step(u0, range(nc), lambda k: range(ns_full + (1 if u0 * nc + k < rem else 0)))
            u0 += 1
        if nu > u0:
            lax.fori_loop(u0, nu, lambda u, c: (step(u, range(nc), lambda k: range(ns_full)), c)[1], 0)
        step(nu, range(st - nu * nc), lambda k: range(ns_full + (1 if nu * nc + k < rem else 0)))

    def issue_streams(streams, rt0, nrt, pattern):
        k = 0
        ncmax = max(s[6] for s in streams)
        for i in range(nrt):
            for c in range(ncmax):
                for (src, dst, sem, sr0, dr0, pc, nc) in streams:
                    if c >= nc:
                        continue
                    ro = (rt0 + i) * 8
                    pltpu.make_async_copy(
                        src.at[pl.ds(_mo(sr0 + ro, 8), 8), pl.ds(c * pc, pc)],
                        dst.at[pl.ds(_mo(dr0 + ro, 8), 8), pl.ds(c * pc, pc)], sem,
                    ).start(priority=pattern[k % len(pattern)])
                    k += 1

    def wait_all(buf, sem):
        pltpu.make_async_copy(buf, buf, sem).wait()

    def kernel(*refs):
        pl.run_scoped(functools.partial(body, *refs), pltpu.SemaphoreType.DMA((NSEM,)))

    def body(x_hbm, c_hbm, b1_hbm, wmod_hbm, wq_hbm, k_hbm, v_hbm, wo_hbm, w1_hbm, w2_hbm,
             o_ref,
             x_v, c_v, b1_v, wmod_v, wq_v, kbuf, vbuf, wo_v, w1_v, w2a_v, w2b_v, w2c_v,
             mod_s, q_s, o_s, s_s, p_s, hh_s, y_s, ab_s, y8_s,
             sems):
        SK = k_hbm.shape[1]
        W = kbuf.shape[2]
        w0 = SK - W
        CW = W // NCH

        def issue_k(g, ch, nch):
            slot = g % 2
            issue_kv(k_hbm, kbuf.at[slot], sems.at[S_K + slot], g * R, w0, W, ch, nch)

        def issue_v(g, ch, nch):
            slot = g % 2
            issue_kv(v_hbm, vbuf.at[slot], sems.at[S_V + slot], g * R, w0, W, ch, nch)

        def loop(n, fn, init=0):
            return lax.fori_loop(0, n, fn, init)

        NWO = HQ * DH // 8
        wo_ns = NWO // wo_st
        wo_streams = [(wo_hbm, wo_v, sems.at[S_WO], 8 * wo_st * m, 8 * wo_st * m, D, 1) for m in range(wo_ns)]

        cp_c = pltpu.make_async_copy(c_hbm, c_v, sems.at[S_C])
        cp_x = pltpu.make_async_copy(x_hbm, x_v, sems.at[S_X])
        cp_b1 = pltpu.make_async_copy(b1_hbm, b1_v, sems.at[S_B1])

        wmod_nc = 6 * D // wmod_pc
        wmod_idx = _flat_order(80 * wmod_nc, wmod_st)
        wq_nc = HQ * DH // wq_pc
        wq_idx = _flat_order(80 * wq_nc, 256 * 128 // wq_pc)

        def small():
            cp_c.start()
            cp_x.start()
            cp_b1.start()
        if pro_loop:
            issue_flat_loop(wmod_hbm, wmod_v, sems.at[S_WMOD], wmod_pc, wmod_nc, 80 * wmod_nc, wmod_st, ppat, small)
        else:
            issue_flat(wmod_hbm, wmod_v, sems.at[S_WMOD], wmod_pc, wmod_nc, wmod_idx[:30], ppat)
            small()
            issue_flat(wmod_hbm, wmod_v, sems.at[S_WMOD], wmod_pc, wmod_nc, wmod_idx[30:], ppat)
            issue_flat(wq_hbm, wq_v, sems.at[S_WQ], wq_pc, wq_nc, wq_idx[:96], ppat)

        cp_c.wait()
        cp_x.wait()
        c = c_v[...].astype(f32)
        sc = (c * jax.nn.sigmoid(c)).astype(bf16)
        x = x_v[...].astype(f32)

        def ln(z):
            m = jnp.mean(z, axis=-1, keepdims=True)
            zc = z - m
            v = jnp.mean(zc * zc, axis=-1, keepdims=True)
            return zc * lax.rsqrt(v + EPS)

        y_s[0:1, :] = ln(x)
        if pro_loop:
            issue_flat_loop(wq_hbm, wq_v, sems.at[S_WQ], wq_pc, wq_nc, 80 * wq_nc, 256 * 128 // wq_pc, ppat)
        else:
            issue_flat(wq_hbm, wq_v, sems.at[S_WQ], wq_pc, wq_nc, wq_idx[96:], ppat)
        wait_all(wmod_v, sems.at[S_WMOD])

        def _mod(ch, cr):
            issue_k(0, ch, 8)
            off = pl.multiple_of(jnp.minimum(ch, 5) * D, 128)
            if wcompute:
                mod_s[:, pl.ds(off, D)] = jnp.dot(sc, wmod_v[:, pl.ds(off, D)], preferred_element_type=f32)
            else:
                mod_s[:, pl.ds(off, D)] = wmod_v[0:1, pl.ds(off, D)].astype(f32)
            return cr
        loop(6, _mod)
        issue_k(0, 6, 8)
        issue_k(0, 7, 8)

        h = (y_s[0:1, :] * (1.0 + mod_s[:, D:2 * D]) + mod_s[:, 0:D]).astype(bf16)
        wait_all(wq_v, sems.at[S_WQ])

        QC = HQ * DH // 8

        def _q(ch, cr):
            issue_v(0, ch, 8)
            off = pl.multiple_of(ch * QC, 128)
            if wcompute:
                q_s[:, pl.ds(off, QC)] = jnp.dot(h, wq_v[:, pl.ds(off, QC)], preferred_element_type=f32) * (DH ** -0.5)
            else:
                q_s[:, pl.ds(off, QC)] = wq_v[0:1, pl.ds(off, QC)].astype(f32)
            return cr
        loop(8, _q)

        row = lax.broadcasted_iota(jnp.int32, (8, R), 0)
        col = lax.broadcasted_iota(jnp.int32, (8, R), 1)
        diag = (col >= row * DH) & (col < (row + 1) * DH)

        def group(g, issue_a, issue_b):
            slot = g % 2
            off = _mo(g * R, 128)
            qg = q_s[:, pl.ds(off, R)]
            qbd = jnp.where(diag, jnp.broadcast_to(qg, (8, R)), 0.0).astype(bf16)
            wait_all(kbuf.at[slot], sems.at[S_K + slot])

            def qk(ch, cr):
                issue_a(ch)
                co = pl.multiple_of(ch * CW, 128)
                if compute:
                    s_s[:, pl.ds(co, CW)] = jnp.dot(qbd, kbuf[slot, :, pl.ds(co, CW)], preferred_element_type=f32)
                else:
                    s_s[:, pl.ds(co, CW)] = kbuf[slot, 0:8, pl.ds(co, CW)].astype(f32)
                return cr
            loop(NCH, qk)

            s = s_s[...]
            m = jnp.max(s, axis=-1, keepdims=True)
            p = jnp.exp(s - m)
            l = jnp.sum(p, axis=-1, keepdims=True)
            p_s[...] = p
            wait_all(vbuf.at[slot], sems.at[S_V + slot])

            def pv(ch, acc):
                issue_b(ch)
                co = pl.multiple_of(ch * CW, 128)
                if compute:
                    return acc + lax.dot_general(p_s[:, pl.ds(co, CW)].astype(bf16), vbuf[slot, :, pl.ds(co, CW)],
                                                 (((1,), (1,)), ((), ())), preferred_element_type=f32)
                else:
                    return acc + vbuf[slot, 0:8, pl.ds(0, R)].astype(f32)
            ov = loop(NCH, pv, jnp.zeros((8, R), f32))
            ov = jnp.where(diag, ov / l, 0.0)
            o_s[:, pl.ds(off, R)] = jnp.sum(ov, axis=0, keepdims=True)

        def main(g, cr):
            group(g, lambda ch: issue_k(g + 1, ch, NCH), lambda ch: issue_v(g + 1, ch, NCH))
            return cr
        loop(NG - 1, main)
        group(NG - 1, lambda ch: issue_streams(wo_streams, ch * wo_tpc, wo_tpc, wpat),
              lambda ch: issue_streams(wo_streams, (NCH + ch) * wo_tpc, wo_tpc, wpat))

        w1_nc = F // w1_pc
        w1_str = [(w1_hbm, w1_v, sems.at[S_W1], 160 * m, 160 * m, w1_pc, w1_nc) for m in range(4)]
        w2a_str = [(w2_hbm, w2a_v, sems.at[S_W2], 384 * m, 256 * m, D, 1) for m in range(4)]
        w2b_str = [(w2_hbm, w2b_v, sems.at[S_W2 + 1], 384 * m + 256, 128 * m, D, 1) for m in range(3)]
        w2c_str = [(w2_hbm, w2c_v, sems.at[S_W2 + 2], 384 * 3 + 256, 0, D, 1)]

        issue_streams(wo_streams, 2 * NCH * wo_tpc, wo_st - 2 * NCH * wo_tpc, wpat)
        issue_flat(wo_hbm, wo_v, sems.at[S_WO], D, 1, list(range(wo_ns * wo_st, NWO)), wpat)
        issue_streams(w1_str, 0, 8, tpat)
        wait_all(wo_v, sems.at[S_WO])

        def wo_dot(m):
            lo = _mo(768 * m, 128)
            if wcompute:
                return jnp.dot(o_s[:, pl.ds(lo, 768)].astype(bf16), wo_v[pl.ds(lo, 768), :], preferred_element_type=f32)
            return wo_v[pl.ds(lo, 16), :][0:1].astype(f32) + o_s[:, pl.ds(lo, 128)][:, 0:1]

        def wo_a(ch, a):
            issue_streams(w1_str, 8 + 2 * ch, 2, tpat)
            return a + wo_dot(ch)
        acc = loop(6, wo_a, jnp.zeros((1, D), f32))

        def wo_b(ch, a):
            issue_streams(w2a_str, 6 * ch, 6, tpat)
            return a + wo_dot(6 + ch)
        acc = loop(2, wo_b, acc)

        x1 = x + mod_s[:, 2 * D:3 * D] * acc
        h2 = (ln(x1) * (1.0 + mod_s[:, 4 * D:5 * D]) + mod_s[:, 3 * D:4 * D]).astype(bf16)
        y_s[0:1, :] = h2.astype(f32)
        y_s[1:2, :] = x1
        issue_streams(w2a_str, 12, 4, tpat)
        cp_b1.wait()
        b1 = b1_v[...].astype(f32)
        hh_s[...] = jnp.concatenate([b1[j:j + 1, :] for j in range(F // 128)], axis=1)
        wait_all(w1_v, sems.at[S_W1])

        def w1_it(ch, cr):
            issue_streams(w2a_str, 16 + 4 * ch, 4, tpat)
            co = pl.multiple_of(ch * 384, 128)
            if wcompute:
                hh = hh_s[:, pl.ds(co, 384)] + jnp.dot(y_s[0:1, :].astype(bf16), w1_v[:, pl.ds(co, 384)],
                                                       preferred_element_type=f32)
            else:
                hh = hh_s[:, pl.ds(co, 384)] + w1_v[0:1, pl.ds(co, 384)].astype(f32)
            sp = jnp.log1p(jnp.exp(-jnp.abs(hh))) + jnp.maximum(hh, 0.0)
            hh_s[:, pl.ds(co, 384)] = hh * jnp.tanh(sp)
            return cr
        loop(4, w1_it)

        issue_streams(w2b_str, 0, 16, tpat)
        if vpu_end:
            issue_streams(w2c_str, 0, c1 // 8, tpat)
            issue_streams([(w2_hbm, w2c_v, sems.at[S_W2 + 3], 384 * 3 + 256, 0, D, 1)], c1 // 8, 16 - c1 // 8, tpat)
            ab_s[...] = jnp.broadcast_to(hh_s[:, 384 * 3 + 256:], (128, 128)).T
        else:
            issue_streams(w2c_str, 0, 16, tpat)

        def dotw(a, wv):
            if wcompute:
                return jnp.dot(a.astype(bf16), wv[...], preferred_element_type=f32)
            return wv[0:1, :].astype(f32) + a[:, 0:1]

        wait_all(w2a_v, sems.at[S_W2])
        act_a = jnp.concatenate([hh_s[:, 384 * m:384 * m + 256] for m in range(4)], axis=1)
        y_s[2:3, :] = dotw(act_a, w2a_v)
        wait_all(w2b_v, sems.at[S_W2 + 1])
        act_b = jnp.concatenate([hh_s[:, 384 * m + 256:384 * m + 384] for m in range(3)], axis=1)
        gb = mod_s[:, 5 * D:6 * D]
        y_s[3:4, :] = y_s[1:2, :] + gb * (y_s[2:3, :] + dotw(act_b, w2b_v))
        if vpu_end:
            def vpu_part(r0, n):
                w = w2c_v[r0:r0 + n, :].astype(f32)
                a = ab_s[r0:r0 + n, :]
                prod = w * jnp.concatenate([a] * (D // 128), axis=1)
                return jnp.sum(prod.reshape(n // 8, 8, D), axis=0)
            wait_all(w2c_v.at[pl.ds(0, c1), :], sems.at[S_W2 + 2])
            y8_s[...] = vpu_part(0, c1)
            wait_all(w2c_v.at[pl.ds(c1, 128 - c1), :], sems.at[S_W2 + 3])
            yc = jnp.sum(y8_s[...] + vpu_part(c1, 128 - c1), axis=0, keepdims=True)
            o_ref[...] = (y_s[3:4, :] + gb * yc).astype(o_ref.dtype)
        else:
            wait_all(w2c_v, sems.at[S_W2 + 2])
            o_ref[...] = (y_s[3:4, :] + gb * dotw(hh_s[:, 384 * 3 + 256:], w2c_v)).astype(o_ref.dtype)

    @jax.jit
    def f(A_x, A_k_cache, A_v_cache, A_wq, A_wo, B_x, B_w1, B_b1, B_w2, c, w_mod):
        B, H, SK, dh = A_k_cache.shape
        W = min(4096, max(256, SK // 4))
        kt = jnp.swapaxes(A_k_cache, 2, 3).reshape(H * dh, SK)
        vt = jnp.swapaxes(A_v_cache, 2, 3).reshape(H * dh, SK)
        x2 = A_x.reshape(1, D)
        b1 = B_b1.reshape(F // 128, 128)
        out = pl.pallas_call(
            kernel,
            out_shape=jax.ShapeDtypeStruct((1, D), A_x.dtype),
            in_specs=[pl.BlockSpec(memory_space=pl.ANY)] * 10,
            out_specs=pl.BlockSpec(memory_space=pltpu.VMEM),
            scratch_shapes=[
                pltpu.VMEM((1, D), bf16), pltpu.VMEM((1, D), bf16), pltpu.VMEM((F // 128, 128), bf16),
                pltpu.VMEM((D, 6 * D), bf16), pltpu.VMEM((D, HQ * DH), bf16),
                pltpu.VMEM((2, R, W), bf16), pltpu.VMEM((2, R, W), bf16),
                pltpu.VMEM((HQ * DH, D), bf16), pltpu.VMEM((D, F), bf16),
                pltpu.VMEM((1024, D), bf16), pltpu.VMEM((384, D), bf16), pltpu.VMEM((128, D), bf16),
                pltpu.VMEM((1, 6 * D), f32), pltpu.VMEM((1, HQ * DH), f32), pltpu.VMEM((1, HQ * DH), f32),
                pltpu.VMEM((8, W), f32), pltpu.VMEM((8, W), f32), pltpu.VMEM((1, F), f32), pltpu.VMEM((8, D), f32),
                pltpu.VMEM((128, 128), f32), pltpu.VMEM((8, D), f32),
            ],
            compiler_params=pltpu.CompilerParams(vmem_limit_bytes=100 * 1024 * 1024, disable_bounds_checks=nobc),
        )(x2, c, b1, w_mod, A_wq, kt, vt, A_wo, B_w1, B_w2)
        return out.reshape(A_x.shape)
    return f


_impl = make(**dict(pro_loop=True, wq_pc=256, wmod_pc=256, wmod_st=128, ppat=(0,)+(1,)*7, split=((32,0),(80,1),(80,1))))


@jax.jit
def pallas_adaLN_cond__sliding_block_cached__dense_activation_mish__decode_kernel(
    A_x: jax.Array,
    A_k_cache: jax.Array,
    A_v_cache: jax.Array,
    A_wq: jax.Array,
    A_wo: jax.Array,
    B_x: jax.Array,
    B_w1: jax.Array,
    B_b1: jax.Array,
    B_w2: jax.Array,
    c: jax.Array,
    w_mod: jax.Array,
):
    return _impl(A_x, A_k_cache, A_v_cache, A_wq, A_wo, B_x, B_w1, B_b1, B_w2, c, w_mod)
```

```python
import functools

import jax
import jax.numpy as jnp
from jax import lax
from jax.experimental import pallas as pl
from jax.experimental.pallas import tpu as pltpu

D = 640
HQ = 32
DH = 192
F = 1536
EPS = 1e-5
f32 = jnp.float32
bf16 = jnp.bfloat16

R = 2 * DH
NG = HQ * DH // R
NCH = 8
KV_SPLIT = ((32, 0), (80, 1), (80, 1))
PRO_PAT = (0, 1, 1, 1, 1, 1, 1, 1)
WO_PAT = (0, 1, 1, 1, 1)
TAIL_PAT = (0, 1, 1, 1)
PRO_PC = 256
PRO_ST = 128
WO_ST = 51
WO_TPC = 3
W1_PC = 512
C2 = 96
C1 = 256 - C2

S_C, S_X, S_B1, S_WMOD, S_WQ, S_K, S_V, S_WO, S_W1, S_W2 = 0, 1, 2, 3, 4, 5, 7, 9, 10, 11
NSEM = S_W2 + 4


def _mo(v, m):
    return v if isinstance(v, int) else pl.multiple_of(v, m)


def _copy(src, dst, sem, sr, dr, rows, sc, dc, cols, priority):
    pltpu.make_async_copy(
        src.at[pl.ds(_mo(sr, 8), rows), pl.ds(_mo(sc, 128), cols)],
        dst.at[pl.ds(_mo(dr, 8), rows), pl.ds(_mo(dc, 128), cols)],
        sem,
    ).start(priority=priority)


def _wait_all(buf, sem):
    pltpu.make_async_copy(buf, buf, sem).wait()


def _issue_kv(src, dst, sem, row0, col0, ch):
    nct = dst.shape[1] // 128
    per = 2 * nct // NCH
    cph = nct // per
    half = ch // cph
    c0 = (ch % cph) * per
    for k in range(per):
        o = 0
        for rows, prio in KV_SPLIT:
            r = half * DH + o
            c = (c0 + k) * 128
            _copy(src, dst, sem, row0 + r, r, rows, col0 + c, c, 128, prio)
            o += rows


def _issue_flat(src, dst, sem, after_first=None):
    nc = src.shape[1] // PRO_PC
    n = src.shape[0] // 8 * nc
    full = n // PRO_ST
    rem = n - full * PRO_ST

    def step(u, nk, nstreams):
        i = 0
        for k in range(nk):
            for m in range(nstreams(k)):
                j0 = PRO_ST * m + k
                r = (j0 // nc + u) * 8
                c = (j0 % nc) * PRO_PC
                _copy(src, dst, sem, r, r, 8, c, c, PRO_PC, PRO_PAT[i % len(PRO_PAT)])
                i += 1

    def rolled(lo, hi, ns):
        def it(u, carry):
            step(u, nc, lambda k: ns)
            return carry
        if hi > lo:
            lax.fori_loop(lo, hi, it, 0)

    def partial(u, nk):
        step(u, nk, lambda k: full + (1 if u * nc + k < rem else 0))

    nu = PRO_ST // nc
    nu_p = rem // nc
    u = 0
    if after_first is not None:
        partial(0, nc)
        after_first()
        u = 1
    rolled(u, nu_p, full + 1)
    u = max(u, nu_p)
    if u == nu_p and rem % nc:
        partial(u, nc)
        u += 1
    rolled(u, nu, full)
    partial(nu, PRO_ST - nu * nc)


def _issue_streams(src, dst, sem, starts, pc, rt0, nrt, pattern):
    i = 0
    for t in range(nrt):
        for c in range(0, src.shape[1], pc):
            for sr, dr in starts:
                r = (rt0 + t) * 8
                _copy(src, dst, sem, sr + r, dr + r, 8, c, c, pc, pattern[i % len(pattern)])
                i += 1


def _layernorm(z):
    m = jnp.mean(z, axis=-1, keepdims=True)
    zc = z - m
    v = jnp.mean(zc * zc, axis=-1, keepdims=True)
    return zc * lax.rsqrt(v + EPS)


def _dot(a, b):
    return jnp.dot(a.astype(bf16), b, preferred_element_type=f32)


def _body(x_hbm, c_hbm, b1_hbm, wmod_hbm, wq_hbm, k_hbm, v_hbm, wo_hbm, w1_hbm, w2_hbm,
          o_ref,
          x_v, c_v, b1_v, wmod_v, wq_v, kbuf, vbuf, wo_v, w1_v, w2a_v, w2b_v, w2c_v,
          mod_s, q_s, o_s, s_s, p_s, hh_s, y_s, ab_s, y8_s,
          sems):
    W = kbuf.shape[2]
    w0 = k_hbm.shape[1] - W
    CW = W // NCH

    def issue_k(g, ch):
        _issue_kv(k_hbm, kbuf.at[g % 2], sems.at[S_K + g % 2], g * R, w0, ch)

    def issue_v(g, ch):
        _issue_kv(v_hbm, vbuf.at[g % 2], sems.at[S_V + g % 2], g * R, w0, ch)

    def loop(n, fn, init=0):
        return lax.fori_loop(0, n, fn, init)

    cp_c = pltpu.make_async_copy(c_hbm, c_v, sems.at[S_C])
    cp_x = pltpu.make_async_copy(x_hbm, x_v, sems.at[S_X])
    cp_b1 = pltpu.make_async_copy(b1_hbm, b1_v, sems.at[S_B1])

    def start_small():
        cp_c.start()
        cp_x.start()
        cp_b1.start()

    _issue_flat(wmod_hbm, wmod_v, sems.at[S_WMOD], start_small)
    cp_c.wait()
    cp_x.wait()
    c = c_v[...].astype(f32)
    sc = c * jax.nn.sigmoid(c)
    x = x_v[...].astype(f32)
    y_s[0:1, :] = _layernorm(x)
    _issue_flat(wq_hbm, wq_v, sems.at[S_WQ])
    _wait_all(wmod_v, sems.at[S_WMOD])

    def mod_it(ch, carry):
        issue_k(0, ch)
        off = pl.multiple_of(ch * D, 128)
        mod_s[:, pl.ds(off, D)] = _dot(sc, wmod_v[:, pl.ds(off, D)])
        return carry
    loop(6, mod_it)
    for ch in range(6, NCH):
        issue_k(0, ch)

    h = y_s[0:1, :] * (1.0 + mod_s[:, D:2 * D]) + mod_s[:, 0:D]
    _wait_all(wq_v, sems.at[S_WQ])
    QC = HQ * DH // NCH

    def q_it(ch, carry):
        issue_v(0, ch)
        off = pl.multiple_of(ch * QC, 128)
        q_s[:, pl.ds(off, QC)] = _dot(h, wq_v[:, pl.ds(off, QC)]) * (DH ** -0.5)
        return carry
    loop(NCH, q_it)

    row = lax.broadcasted_iota(jnp.int32, (8, R), 0)
    col = lax.broadcasted_iota(jnp.int32, (8, R), 1)
    diag = (col >= row * DH) & (col < (row + 1) * DH)

    def group(g, issue_a, issue_b):
        slot = g % 2
        off = _mo(g * R, 128)
        qbd = jnp.where(diag, jnp.broadcast_to(q_s[:, pl.ds(off, R)], (8, R)), 0.0).astype(bf16)
        _wait_all(kbuf.at[slot], sems.at[S_K + slot])

        def qk(ch, carry):
            issue_a(ch)
            co = pl.multiple_of(ch * CW, 128)
            s_s[:, pl.ds(co, CW)] = jnp.dot(qbd, kbuf[slot, :, pl.ds(co, CW)], preferred_element_type=f32)
            return carry
        loop(NCH, qk)

        s = s_s[...]
        p = jnp.exp(s - jnp.max(s, axis=-1, keepdims=True))
        l = jnp.sum(p, axis=-1, keepdims=True)
        p_s[...] = p
        _wait_all(vbuf.at[slot], sems.at[S_V + slot])

        def pv(ch, acc):
            issue_b(ch)
            co = pl.multiple_of(ch * CW, 128)
            return acc + lax.dot_general(p_s[:, pl.ds(co, CW)].astype(bf16), vbuf[slot, :, pl.ds(co, CW)],
                                         (((1,), (1,)), ((), ())), preferred_element_type=f32)
        ov = loop(NCH, pv, jnp.zeros((8, R), f32))
        o_s[:, pl.ds(off, R)] = jnp.sum(jnp.where(diag, ov / l, 0.0), axis=0, keepdims=True)

    def main(g, carry):
        group(g, lambda ch: issue_k(g + 1, ch), lambda ch: issue_v(g + 1, ch))
        return carry
    loop(NG - 1, main)

    nwo = HQ * DH // 8
    wo_starts = [(8 * WO_ST * m,) * 2 for m in range(nwo // WO_ST)]

    def issue_wo(rt0, nrt):
        _issue_streams(wo_hbm, wo_v, sems.at[S_WO], wo_starts, D, rt0, nrt, WO_PAT)

    group(NG - 1, lambda ch: issue_wo(ch * WO_TPC, WO_TPC), lambda ch: issue_wo((NCH + ch) * WO_TPC, WO_TPC))

    def issue_w1(rt0, nrt):
        _issue_streams(w1_hbm, w1_v, sems.at[S_W1], [(160 * m,) * 2 for m in range(4)], W1_PC, rt0, nrt, TAIL_PAT)

    def issue_w2a(rt0, nrt):
        _issue_streams(w2_hbm, w2a_v, sems.at[S_W2], [(384 * m, 256 * m) for m in range(4)], D, rt0, nrt, TAIL_PAT)

    issue_wo(2 * NCH * WO_TPC, WO_ST - 2 * NCH * WO_TPC)
    last = len(wo_starts) * WO_ST
    _issue_streams(wo_hbm, wo_v, sems.at[S_WO], [(8 * last,) * 2], D, 0, nwo - last, WO_PAT)
    issue_w1(0, 8)
    _wait_all(wo_v, sems.at[S_WO])

    def wo_dot(m):
        lo = _mo(768 * m, 128)
        return _dot(o_s[:, pl.ds(lo, 768)], wo_v[pl.ds(lo, 768), :])

    def wo_a(ch, acc):
        issue_w1(8 + 2 * ch, 2)
        return acc + wo_dot(ch)
    att = loop(6, wo_a, jnp.zeros((1, D), f32))

    def wo_b(ch, acc):
        issue_w2a(6 * ch, 6)
        return acc + wo_dot(6 + ch)
    att = loop(2, wo_b, att)

    x1 = x + mod_s[:, 2 * D:3 * D] * att
    y_s[0:1, :] = _layernorm(x1) * (1.0 + mod_s[:, 4 * D:5 * D]) + mod_s[:, 3 * D:4 * D]
    y_s[1:2, :] = x1
    issue_w2a(12, 4)
    cp_b1.wait()
    b1 = b1_v[...].astype(f32)
    hh_s[...] = jnp.concatenate([b1[j:j + 1, :] for j in range(F // 128)], axis=1)
    _wait_all(w1_v, sems.at[S_W1])

    def w1_it(ch, carry):
        issue_w2a(16 + 4 * ch, 4)
        co = pl.multiple_of(ch * 384, 128)
        hh = hh_s[:, pl.ds(co, 384)] + _dot(y_s[0:1, :], w1_v[:, pl.ds(co, 384)])
        sp = jnp.log1p(jnp.exp(-jnp.abs(hh))) + jnp.maximum(hh, 0.0)
        hh_s[:, pl.ds(co, 384)] = hh * jnp.tanh(sp)
        return carry
    loop(4, w1_it)

    _issue_streams(w2_hbm, w2b_v, sems.at[S_W2 + 1], [(384 * m + 256, 128 * m) for m in range(2)], D, 0, 16, TAIL_PAT)
    for j in range(32):
        t, i = j // 2, j % 2
        _copy(w2_hbm, w2c_v, sems.at[S_W2 + (2 if 8 * j < C1 else 3)], 384 * (2 + i) + 256 + 8 * t, 8 * j, 8,
              0, 0, D, TAIL_PAT[j % len(TAIL_PAT)])
    for i in range(2):
        lo = 384 * (2 + i) + 256
        abt = jnp.broadcast_to(hh_s[:, lo:lo + 128], (128, 128)).T
        for t in range(16):
            ab_s[8 * (2 * t + i):8 * (2 * t + i) + 8, :] = abt[8 * t:8 * t + 8, :]

    _wait_all(w2a_v, sems.at[S_W2])
    act_a = jnp.concatenate([hh_s[:, 384 * m:384 * m + 256] for m in range(4)], axis=1)
    y_s[2:3, :] = _dot(act_a, w2a_v[...])
    _wait_all(w2b_v, sems.at[S_W2 + 1])
    act_b = jnp.concatenate([hh_s[:, 384 * m + 256:384 * m + 384] for m in range(2)], axis=1)
    gb = mod_s[:, 5 * D:6 * D]
    y_s[3:4, :] = y_s[1:2, :] + gb * (y_s[2:3, :] + _dot(act_b, w2b_v[...]))

    def vpu_part(r0, n):
        prod = w2c_v[r0:r0 + n, :].astype(f32) * jnp.concatenate([ab_s[r0:r0 + n, :]] * (D // 128), axis=1)
        return jnp.sum(prod.reshape(n // 8, 8, D), axis=0)

    _wait_all(w2c_v.at[pl.ds(0, C1), :], sems.at[S_W2 + 2])
    y8_s[...] = vpu_part(0, C1)
    _wait_all(w2c_v.at[pl.ds(C1, C2), :], sems.at[S_W2 + 3])
    yc = jnp.sum(y8_s[...] + vpu_part(C1, C2), axis=0, keepdims=True)
    o_ref[...] = (y_s[3:4, :] + gb * yc).astype(o_ref.dtype)


def _kernel(*refs):
    pl.run_scoped(functools.partial(_body, *refs), pltpu.SemaphoreType.DMA((NSEM,)))


@jax.jit
def pallas_adaLN_cond__sliding_block_cached__dense_activation_mish__decode_kernel(
    A_x: jax.Array,
    A_k_cache: jax.Array,
    A_v_cache: jax.Array,
    A_wq: jax.Array,
    A_wo: jax.Array,
    B_x: jax.Array,
    B_w1: jax.Array,
    B_b1: jax.Array,
    B_w2: jax.Array,
    c: jax.Array,
    w_mod: jax.Array,
):
    _, H, SK, dh = A_k_cache.shape
    W = min(4096, max(256, SK // 4))
    kt = jnp.swapaxes(A_k_cache, 2, 3).reshape(H * dh, SK)
    vt = jnp.swapaxes(A_v_cache, 2, 3).reshape(H * dh, SK)
    out = pl.pallas_call(
        _kernel,
        out_shape=jax.ShapeDtypeStruct((1, D), A_x.dtype),
        in_specs=[pl.BlockSpec(memory_space=pl.ANY)] * 10,
        out_specs=pl.BlockSpec(memory_space=pltpu.VMEM),
        scratch_shapes=[
            pltpu.VMEM((1, D), bf16), pltpu.VMEM((1, D), bf16), pltpu.VMEM((F // 128, 128), bf16),
            pltpu.VMEM((D, 6 * D), bf16), pltpu.VMEM((D, HQ * DH), bf16),
            pltpu.VMEM((2, R, W), bf16), pltpu.VMEM((2, R, W), bf16),
            pltpu.VMEM((HQ * DH, D), bf16), pltpu.VMEM((D, F), bf16),
            pltpu.VMEM((1024, D), bf16), pltpu.VMEM((256, D), bf16), pltpu.VMEM((256, D), bf16),
            pltpu.VMEM((1, 6 * D), f32), pltpu.VMEM((1, HQ * DH), f32), pltpu.VMEM((1, HQ * DH), f32),
            pltpu.VMEM((8, W), f32), pltpu.VMEM((8, W), f32), pltpu.VMEM((1, F), f32), pltpu.VMEM((8, D), f32),
            pltpu.VMEM((256, 128), f32), pltpu.VMEM((8, D), f32),
        ],
        compiler_params=pltpu.CompilerParams(vmem_limit_bytes=64 * 1024 * 1024, disable_bounds_checks=True),
    )(A_x.reshape(1, D), c, B_b1.reshape(F // 128, 128), w_mod, A_wq, kt, vt, A_wo, B_w1, B_w2)
    return out.reshape(A_x.shape)
```

```python
import functools

import jax
import jax.numpy as jnp
from jax import lax
from jax.experimental import pallas as pl
from jax.experimental.pallas import tpu as pltpu

D = 640
HQ = 32
DH = 192
F = 1536
EPS = 1e-5
f32 = jnp.float32
bf16 = jnp.bfloat16

R = 2 * DH
NG = HQ * DH // R
NCH = 8
KV_SPLIT = ((32, 0), (160, 1))
PRO_PAT = (0, 1, 1, 1, 1, 1, 1, 1)
WO_PAT = (0, 1, 1, 1, 1)
TAIL_PAT = (0, 1, 1, 1)
PRO_PC = 256
PRO_ST = 128
WO_ST = 51
WO_TPC = 3
W1_PC = 512
CS = (160, 64, 32)

S_C, S_X, S_B1, S_WMOD, S_WQ, S_K, S_V, S_WO, S_W1, S_W2 = 0, 1, 2, 3, 4, 5, 7, 9, 10, 11
NSEM = S_W2 + 2 + len(CS)


def _mo(v, m):
    return v if isinstance(v, int) else pl.multiple_of(v, m)


def _copy(src, dst, sem, sr, dr, rows, sc, dc, cols, priority):
    pltpu.make_async_copy(
        src.at[pl.ds(_mo(sr, 8), rows), pl.ds(_mo(sc, 128), cols)],
        dst.at[pl.ds(_mo(dr, 8), rows), pl.ds(_mo(dc, 128), cols)],
        sem,
    ).start(priority=priority)


def _wait_all(buf, sem):
    pltpu.make_async_copy(buf, buf, sem).wait()


def _issue_kv(src, dst, sem, row0, col0, ch):
    nct = dst.shape[1] // 128
    per = 2 * nct // NCH
    cph = nct // per
    half = ch // cph
    c0 = (ch % cph) * per
    for k in range(per):
        o = 0
        for rows, prio in KV_SPLIT:
            r = half * DH + o
            c = (c0 + k) * 128
            _copy(src, dst, sem, row0 + r, r, rows, col0 + c, c, 128, prio)
            o += rows


def _issue_flat(src, dst, sem, after_first=None):
    nc = src.shape[1] // PRO_PC
    n = src.shape[0] // 8 * nc
    full = n // PRO_ST
    rem = n - full * PRO_ST

    def step(u, nk, nstreams):
        i = 0
        for k in range(nk):
            for m in range(nstreams(k)):
                j0 = PRO_ST * m + k
                r = (j0 // nc + u) * 8
                c = (j0 % nc) * PRO_PC
                _copy(src, dst, sem, r, r, 8, c, c, PRO_PC, PRO_PAT[i % len(PRO_PAT)])
                i += 1

    def rolled(lo, hi, ns):
        def it(u, carry):
            step(u, nc, lambda k: ns)
            return carry
        if hi > lo:
            lax.fori_loop(lo, hi, it, 0)

    def partial(u, nk):
        step(u, nk, lambda k: full + (1 if u * nc + k < rem else 0))

    nu = PRO_ST // nc
    nu_p = rem // nc
    u = 0
    if after_first is not None:
        partial(0, nc)
        after_first()
        u = 1
    rolled(u, nu_p, full + 1)
    u = max(u, nu_p)
    if u == nu_p and rem % nc:
        partial(u, nc)
        u += 1
    rolled(u, nu, full)
    partial(nu, PRO_ST - nu * nc)


def _issue_streams(src, dst, sem, starts, pc, rt0, nrt, pattern):
    i = 0
    for t in range(nrt):
        for c in range(0, src.shape[1], pc):
            for sr, dr in starts:
                r = (rt0 + t) * 8
                _copy(src, dst, sem, sr + r, dr + r, 8, c, c, pc, pattern[i % len(pattern)])
                i += 1


def _layernorm(z):
    m = jnp.mean(z, axis=-1, keepdims=True)
    zc = z - m
    v = jnp.mean(zc * zc, axis=-1, keepdims=True)
    return zc * lax.rsqrt(v + EPS)


def _dot(a, b):
    return jnp.dot(a.astype(bf16), b, preferred_element_type=f32)


def _body(x_hbm, c_hbm, b1_hbm, wmod_hbm, wq_hbm, k_hbm, v_hbm, wo_hbm, w1_hbm, w2_hbm,
          o_ref,
          x_v, c_v, b1_v, wmod_v, wq_v, kbuf, vbuf, wo_v, w1_v, w2a_v, w2b_v, w2c_v,
          mod_s, q_s, o_s, s_s, p_s, hh_s, y_s, ab_s, y8_s,
          sems):
    W = kbuf.shape[2]
    w0 = k_hbm.shape[1] - W
    CW = W // NCH

    def issue_k(g, ch):
        _issue_kv(k_hbm, kbuf.at[g % 2], sems.at[S_K + g % 2], g * R, w0, ch)

    def issue_v(g, ch):
        _issue_kv(v_hbm, vbuf.at[g % 2], sems.at[S_V + g % 2], g * R, w0, ch)

    def loop(n, fn, init=0):
        return lax.fori_loop(0, n, fn, init)

    cp_c = pltpu.make_async_copy(c_hbm, c_v, sems.at[S_C])
    cp_x = pltpu.make_async_copy(x_hbm, x_v, sems.at[S_X])
    cp_b1 = pltpu.make_async_copy(b1_hbm, b1_v, sems.at[S_B1])

    def start_small():
        cp_c.start()
        cp_x.start()
        cp_b1.start()

    _issue_flat(wmod_hbm, wmod_v, sems.at[S_WMOD], start_small)
    cp_c.wait()
    cp_x.wait()
    c = c_v[...].astype(f32)
    sc = c * jax.nn.sigmoid(c)
    x = x_v[...].astype(f32)
    y_s[0:1, :] = _layernorm(x)
    _issue_flat(wq_hbm, wq_v, sems.at[S_WQ])
    _wait_all(wmod_v, sems.at[S_WMOD])

    def mod_it(ch, carry):
        issue_k(0, ch)
        off = pl.multiple_of(ch * D, 128)
        mod_s[:, pl.ds(off, D)] = _dot(sc, wmod_v[:, pl.ds(off, D)])
        return carry
    loop(6, mod_it)
    for ch in range(6, NCH):
        issue_k(0, ch)

    h = y_s[0:1, :] * (1.0 + mod_s[:, D:2 * D]) + mod_s[:, 0:D]
    _wait_all(wq_v, sems.at[S_WQ])
    QC = HQ * DH // NCH

    def q_it(ch, carry):
        issue_v(0, ch)
        off = pl.multiple_of(ch * QC, 128)
        q_s[:, pl.ds(off, QC)] = _dot(h, wq_v[:, pl.ds(off, QC)]) * (DH ** -0.5)
        return carry
    loop(NCH, q_it)

    row = lax.broadcasted_iota(jnp.int32, (8, R), 0)
    col = lax.broadcasted_iota(jnp.int32, (8, R), 1)
    diag = (col >= row * DH) & (col < (row + 1) * DH)

    def group(g, issue_a, issue_b):
        slot = g % 2
        off = _mo(g * R, 128)
        qbd = jnp.where(diag, jnp.broadcast_to(q_s[:, pl.ds(off, R)], (8, R)), 0.0).astype(bf16)
        _wait_all(kbuf.at[slot], sems.at[S_K + slot])

        def qk(ch, carry):
            issue_a(ch)
            co = pl.multiple_of(ch * CW, 128)
            s_s[:, pl.ds(co, CW)] = jnp.dot(qbd, kbuf[slot, :, pl.ds(co, CW)], preferred_element_type=f32)
            return carry
        loop(NCH, qk)

        s = s_s[...]
        p = jnp.exp(s - jnp.max(s, axis=-1, keepdims=True))
        l = jnp.sum(p, axis=-1, keepdims=True)
        p_s[...] = p
        _wait_all(vbuf.at[slot], sems.at[S_V + slot])

        def pv(ch, acc):
            issue_b(ch)
            co = pl.multiple_of(ch * CW, 128)
            return acc + lax.dot_general(p_s[:, pl.ds(co, CW)].astype(bf16), vbuf[slot, :, pl.ds(co, CW)],
                                         (((1,), (1,)), ((), ())), preferred_element_type=f32)
        ov = loop(NCH, pv, jnp.zeros((8, R), f32))
        o_s[:, pl.ds(off, R)] = jnp.sum(jnp.where(diag, ov / l, 0.0), axis=0, keepdims=True)

    def main(g, carry):
        group(g, lambda ch: issue_k(g + 1, ch), lambda ch: issue_v(g + 1, ch))
        return carry
    loop(NG - 1, main)

    nwo = HQ * DH // 8
    wo_starts = [(8 * WO_ST * m,) * 2 for m in range(nwo // WO_ST)]

    def issue_wo(rt0, nrt):
        _issue_streams(wo_hbm, wo_v, sems.at[S_WO], wo_starts, D, rt0, nrt, WO_PAT)

    group(NG - 1, lambda ch: issue_wo(ch * WO_TPC, WO_TPC), lambda ch: issue_wo((NCH + ch) * WO_TPC, WO_TPC))

    def issue_w1(rt0, nrt):
        _issue_streams(w1_hbm, w1_v, sems.at[S_W1], [(160 * m,) * 2 for m in range(4)], W1_PC, rt0, nrt, TAIL_PAT)

    def issue_w2a(rt0, nrt):
        _issue_streams(w2_hbm, w2a_v, sems.at[S_W2], [(384 * m, 256 * m) for m in range(4)], D, rt0, nrt, TAIL_PAT)

    issue_wo(2 * NCH * WO_TPC, WO_ST - 2 * NCH * WO_TPC)
    last = len(wo_starts) * WO_ST
    _issue_streams(wo_hbm, wo_v, sems.at[S_WO], [(8 * last,) * 2], D, 0, nwo - last, WO_PAT)
    issue_w1(0, 8)
    _wait_all(wo_v, sems.at[S_WO])

    def wo_dot(m):
        lo = _mo(768 * m, 128)
        return _dot(o_s[:, pl.ds(lo, 768)], wo_v[pl.ds(lo, 768), :])

    def wo_a(ch, acc):
        issue_w1(8 + 2 * ch, 2)
        return acc + wo_dot(ch)
    att = loop(6, wo_a, jnp.zeros((1, D), f32))

    def wo_b(ch, acc):
        issue_w2a(6 * ch, 6)
        return acc + wo_dot(6 + ch)
    att = loop(2, wo_b, att)

    x1 = x + mod_s[:, 2 * D:3 * D] * att
    y_s[0:1, :] = _layernorm(x1) * (1.0 + mod_s[:, 4 * D:5 * D]) + mod_s[:, 3 * D:4 * D]
    y_s[1:2, :] = x1
    issue_w2a(12, 4)
    cp_b1.wait()
    b1 = b1_v[...].astype(f32)
    hh_s[...] = jnp.concatenate([b1[j:j + 1, :] for j in range(F // 128)], axis=1)
    _wait_all(w1_v, sems.at[S_W1])

    def w1_it(ch, carry):
        issue_w2a(16 + 4 * ch, 4)
        co = pl.multiple_of(ch * 384, 128)
        hh = hh_s[:, pl.ds(co, 384)] + _dot(y_s[0:1, :], w1_v[:, pl.ds(co, 384)])
        sp = jnp.log1p(jnp.exp(-jnp.abs(hh))) + jnp.maximum(hh, 0.0)
        hh_s[:, pl.ds(co, 384)] = hh * jnp.tanh(sp)
        return carry
    loop(4, w1_it)

    _issue_streams(w2_hbm, w2b_v, sems.at[S_W2 + 1], [(384 * m + 256, 128 * m) for m in range(2)], D, 0, 16, TAIL_PAT)
    for j in range(32):
        t, i = j // 2, j % 2
        part = sum(1 for e in range(1, len(CS)) if 8 * j >= sum(CS[:e]))
        _copy(w2_hbm, w2c_v, sems.at[S_W2 + 2 + part], 384 * (2 + i) + 256 + 8 * t, 8 * j, 8,
              0, 0, D, TAIL_PAT[j % len(TAIL_PAT)])
    for i in range(2):
        lo = 384 * (2 + i) + 256
        abt = jnp.broadcast_to(hh_s[:, lo:lo + 128], (128, 128)).T
        for t in range(16):
            ab_s[8 * (2 * t + i):8 * (2 * t + i) + 8, :] = abt[8 * t:8 * t + 8, :]

    _wait_all(w2a_v, sems.at[S_W2])
    act_a = jnp.concatenate([hh_s[:, 384 * m:384 * m + 256] for m in range(4)], axis=1)
    y_s[2:3, :] = _dot(act_a, w2a_v[...])
    _wait_all(w2b_v, sems.at[S_W2 + 1])
    act_b = jnp.concatenate([hh_s[:, 384 * m + 256:384 * m + 384] for m in range(2)], axis=1)
    gb = mod_s[:, 5 * D:6 * D]
    y_s[3:4, :] = y_s[1:2, :] + gb * (y_s[2:3, :] + _dot(act_b, w2b_v[...]))

    def vpu_part(r0, n, acc):
        for r in range(r0, r0 + n, 16):
            prod = w2c_v[r:r + 16, :].astype(f32) * jnp.concatenate([ab_s[r:r + 16, :]] * (D // 128), axis=1)
            pr = prod[0:8, :] + prod[8:16, :]
            acc = pr if acc is None else acc + pr
        return acc

    r0 = 0
    for e, n in enumerate(CS):
        _wait_all(w2c_v.at[pl.ds(r0, n), :], sems.at[S_W2 + 2 + e])
        acc = vpu_part(r0, n, None if e == 0 else y8_s[...])
        if e + 1 < len(CS):
            y8_s[...] = acc
        r0 += n
    o_ref[...] = (y_s[3:4, :] + gb * jnp.sum(acc, axis=0, keepdims=True)).astype(o_ref.dtype)


def _kernel(*refs):
    pl.run_scoped(functools.partial(_body, *refs), pltpu.SemaphoreType.DMA((NSEM,)))


@jax.jit
def pallas_adaLN_cond__sliding_block_cached__dense_activation_mish__decode_kernel(
    A_x: jax.Array,
    A_k_cache: jax.Array,
    A_v_cache: jax.Array,
    A_wq: jax.Array,
    A_wo: jax.Array,
    B_x: jax.Array,
    B_w1: jax.Array,
    B_b1: jax.Array,
    B_w2: jax.Array,
    c: jax.Array,
    w_mod: jax.Array,
):
    _, H, SK, dh = A_k_cache.shape
    W = min(4096, max(256, SK // 4))
    kt = jnp.swapaxes(A_k_cache, 2, 3).reshape(H * dh, SK)
    vt = jnp.swapaxes(A_v_cache, 2, 3).reshape(H * dh, SK)
    out = pl.pallas_call(
        _kernel,
        out_shape=jax.ShapeDtypeStruct((1, D), A_x.dtype),
        in_specs=[pl.BlockSpec(memory_space=pl.ANY)] * 10,
        out_specs=pl.BlockSpec(memory_space=pltpu.VMEM),
        scratch_shapes=[
            pltpu.VMEM((1, D), bf16), pltpu.VMEM((1, D), bf16), pltpu.VMEM((F // 128, 128), bf16),
            pltpu.VMEM((D, 6 * D), bf16), pltpu.VMEM((D, HQ * DH), bf16),
            pltpu.VMEM((2, R, W), bf16), pltpu.VMEM((2, R, W), bf16),
            pltpu.VMEM((HQ * DH, D), bf16), pltpu.VMEM((D, F), bf16),
            pltpu.VMEM((1024, D), bf16), pltpu.VMEM((256, D), bf16), pltpu.VMEM((256, D), bf16),
            pltpu.VMEM((1, 6 * D), f32), pltpu.VMEM((1, HQ * DH), f32), pltpu.VMEM((1, HQ * DH), f32),
            pltpu.VMEM((8, W), f32), pltpu.VMEM((8, W), f32), pltpu.VMEM((1, F), f32), pltpu.VMEM((8, D), f32),
            pltpu.VMEM((256, 128), f32), pltpu.VMEM((8, D), f32),
        ],
        compiler_params=pltpu.CompilerParams(vmem_limit_bytes=64 * 1024 * 1024, disable_bounds_checks=True),
    )(A_x.reshape(1, D), c, B_b1.reshape(F // 128, 128), w_mod, A_wq, kt, vt, A_wo, B_w1, B_w2)
    return out.reshape(A_x.shape)
```

```python
import functools

import jax
import jax.numpy as jnp
from jax import lax
from jax.experimental import pallas as pl
from jax.experimental.pallas import tpu as pltpu

D = 640
HQ = 32
DH = 192
F = 1536
EPS = 1e-5
f32 = jnp.float32
bf16 = jnp.bfloat16

R = 2 * DH
NG = HQ * DH // R
NCH = 8
KV_SPLIT = ((32, 0), (160, 1))
PRO_PAT = (0, 1, 1, 1, 1, 1, 1)
WO_PAT = (0, 1, 1, 1, 1, 1, 1)
TAIL_PAT = (0, 1, 1, 1)
PRO_PC = 256
PRO_ST = 128
WO_TPC = 3
W1_PC = 512
CS = (160, 64, 32)

S_C, S_X, S_B1, S_WMOD, S_WQ, S_K, S_V, S_WO, S_W1, S_W2 = 0, 1, 2, 3, 4, 5, 7, 9, 10, 11
NSEM = S_W2 + 2 + len(CS)


def _mo(v, m):
    return v if isinstance(v, int) else pl.multiple_of(v, m)


def _copy(src, dst, sem, sr, dr, rows, sc, dc, cols, priority):
    pltpu.make_async_copy(
        src.at[pl.ds(_mo(sr, 8), rows), pl.ds(_mo(sc, 128), cols)],
        dst.at[pl.ds(_mo(dr, 8), rows), pl.ds(_mo(dc, 128), cols)],
        sem,
    ).start(priority=priority)


def _wait_all(buf, sem):
    pltpu.make_async_copy(buf, buf, sem).wait()


def _issue_kv(src, dst, sem, row0, col0, ch):
    nct = dst.shape[1] // 128
    per = 2 * nct // NCH
    cph = nct // per
    half = ch // cph
    c0 = (ch % cph) * per
    for k in range(per):
        o = 0
        for rows, prio in KV_SPLIT:
            r = half * DH + o
            c = (c0 + k) * 128
            _copy(src, dst, sem, row0 + r, r, rows, col0 + c, c, 128, prio)
            o += rows


def _issue_flat(src, dst, sem, after_first=None):
    nc = src.shape[1] // PRO_PC
    n = src.shape[0] // 8 * nc
    full = n // PRO_ST
    rem = n - full * PRO_ST

    def step(u, nk, nstreams):
        i = 0
        for k in range(nk):
            for m in range(nstreams(k)):
                j0 = PRO_ST * m + k
                r = (j0 // nc + u) * 8
                c = (j0 % nc) * PRO_PC
                _copy(src, dst, sem, r, r, 8, c, c, PRO_PC, PRO_PAT[i % len(PRO_PAT)])
                i += 1

    def rolled(lo, hi, ns):
        def it(u, carry):
            step(u, nc, lambda k: ns)
            return carry
        if hi > lo:
            lax.fori_loop(lo, hi, it, 0)

    def partial(u, nk):
        step(u, nk, lambda k: full + (1 if u * nc + k < rem else 0))

    nu = PRO_ST // nc
    nu_p = rem // nc
    u = 0
    if after_first is not None:
        partial(0, nc)
        after_first()
        u = 1
    rolled(u, nu_p, full + 1)
    u = max(u, nu_p)
    if u == nu_p and rem % nc:
        partial(u, nc)
        u += 1
    rolled(u, nu, full)
    partial(nu, PRO_ST - nu * nc)


def _issue_streams(src, dst, sem, starts, pc, rt0, nrt, pattern):
    i = 0
    for t in range(nrt):
        for c in range(0, src.shape[1], pc):
            for sr, dr in starts:
                r = (rt0 + t) * 8
                _copy(src, dst, sem, sr + r, dr + r, 8, c, c, pc, pattern[i % len(pattern)])
                i += 1


def _wo_pieces(lo, hi):
    out = []
    for m in range(HQ * DH // 8 * 5 // 256):
        pos, end = 256 * m, 256 * (m + 1)
        while pos < end:
            nxt = min(end, pos - pos % 5 + (2 if pos % 5 < 2 else 5))
            cut = pos % 5 in (0, 2)
            off = pos - 256 * m if cut else 255
            if lo <= off < hi:
                out.append((off // 2, m, pos, nxt - pos))
            pos = nxt
    return [(p, n) for _, _, p, n in sorted(out)]


def _layernorm(z):
    m = jnp.mean(z, axis=-1, keepdims=True)
    zc = z - m
    v = jnp.mean(zc * zc, axis=-1, keepdims=True)
    return zc * lax.rsqrt(v + EPS)


def _dot(a, b):
    return jnp.dot(a.astype(bf16), b, preferred_element_type=f32)


def _body(x_hbm, c_hbm, b1_hbm, wmod_hbm, wq_hbm, k_hbm, v_hbm, wo_hbm, w1_hbm, w2_hbm,
          o_ref,
          x_v, c_v, b1_v, wmod_v, wq_v, kbuf, vbuf, wo_v, w1_v, w2a_v, w2b_v, w2c_v,
          mod_s, q_s, o_s, s_s, p_s, hh_s, y_s, ab_s, y8_s,
          sems):
    W = kbuf.shape[2]
    w0 = k_hbm.shape[1] - W
    CW = W // NCH

    def issue_k(g, ch):
        _issue_kv(k_hbm, kbuf.at[g % 2], sems.at[S_K + g % 2], g * R, w0, ch)

    def issue_v(g, ch):
        _issue_kv(v_hbm, vbuf.at[g % 2], sems.at[S_V + g % 2], g * R, w0, ch)

    def loop(n, fn, init=0):
        return lax.fori_loop(0, n, fn, init)

    cp_c = pltpu.make_async_copy(c_hbm, c_v, sems.at[S_C])
    cp_x = pltpu.make_async_copy(x_hbm, x_v, sems.at[S_X])
    cp_b1 = pltpu.make_async_copy(b1_hbm, b1_v, sems.at[S_B1])

    def start_small():
        cp_c.start()
        cp_x.start()
        cp_b1.start()

    _issue_flat(wmod_hbm, wmod_v, sems.at[S_WMOD], start_small)
    cp_c.wait()
    cp_x.wait()
    c = c_v[...].astype(f32)
    sc = c * jax.nn.sigmoid(c)
    x = x_v[...].astype(f32)
    y_s[0:1, :] = _layernorm(x)
    _issue_flat(wq_hbm, wq_v, sems.at[S_WQ])
    _wait_all(wmod_v, sems.at[S_WMOD])

    def mod_it(ch, carry):
        issue_k(0, ch)
        off = pl.multiple_of(ch * D, 128)
        mod_s[:, pl.ds(off, D)] = _dot(sc, wmod_v[:, pl.ds(off, D)])
        return carry
    loop(6, mod_it)
    for ch in range(6, NCH):
        issue_k(0, ch)

    h = y_s[0:1, :] * (1.0 + mod_s[:, D:2 * D]) + mod_s[:, 0:D]
    _wait_all(wq_v, sems.at[S_WQ])
    QC = HQ * DH // NCH

    def q_it(ch, carry):
        issue_v(0, ch)
        off = pl.multiple_of(ch * QC, 128)
        q_s[:, pl.ds(off, QC)] = _dot(h, wq_v[:, pl.ds(off, QC)]) * (DH ** -0.5)
        return carry
    loop(NCH, q_it)

    row = lax.broadcasted_iota(jnp.int32, (8, R), 0)
    col = lax.broadcasted_iota(jnp.int32, (8, R), 1)
    diag = (col >= row * DH) & (col < (row + 1) * DH)

    def group(g, issue_a, issue_b):
        slot = g % 2
        off = _mo(g * R, 128)
        qbd = jnp.where(diag, jnp.broadcast_to(q_s[:, pl.ds(off, R)], (8, R)), 0.0).astype(bf16)
        _wait_all(kbuf.at[slot], sems.at[S_K + slot])

        def qk(ch, carry):
            issue_a(ch)
            co = pl.multiple_of(ch * CW, 128)
            s_s[:, pl.ds(co, CW)] = jnp.dot(qbd, kbuf[slot, :, pl.ds(co, CW)], preferred_element_type=f32)
            return carry
        loop(NCH, qk)

        s = s_s[...]
        p = jnp.exp(s - jnp.max(s, axis=-1, keepdims=True))
        l = jnp.sum(p, axis=-1, keepdims=True)
        p_s[...] = p
        _wait_all(vbuf.at[slot], sems.at[S_V + slot])

        def pv(ch, acc):
            issue_b(ch)
            co = pl.multiple_of(ch * CW, 128)
            return acc + lax.dot_general(p_s[:, pl.ds(co, CW)].astype(bf16), vbuf[slot, :, pl.ds(co, CW)],
                                         (((1,), (1,)), ((), ())), preferred_element_type=f32)
        ov = loop(NCH, pv, jnp.zeros((8, R), f32))
        o_s[:, pl.ds(off, R)] = jnp.sum(jnp.where(diag, ov / l, 0.0), axis=0, keepdims=True)

    def main(g, carry):
        group(g, lambda ch: issue_k(g + 1, ch), lambda ch: issue_v(g + 1, ch))
        return carry
    loop(NG - 1, main)

    def issue_wo(u, lo, hi):
        for i, (p, n) in enumerate(_wo_pieces(lo, hi)):
            r = (p // 5 + u) * 8
            c = p % 5 * 128
            _copy(wo_hbm, wo_v, sems.at[S_WO], r, r, 8, c, c, n * 128, WO_PAT[i % len(WO_PAT)])

    group(NG - 1, lambda ch: issue_wo(ch * WO_TPC, 0, 5 * WO_TPC),
          lambda ch: issue_wo((NCH + ch) * WO_TPC, 0, 5 * WO_TPC))

    def issue_w1(rt0, nrt):
        _issue_streams(w1_hbm, w1_v, sems.at[S_W1], [(160 * m,) * 2 for m in range(4)], W1_PC, rt0, nrt, TAIL_PAT)

    def issue_w2a(rt0, nrt):
        _issue_streams(w2_hbm, w2a_v, sems.at[S_W2], [(384 * m, 256 * m) for m in range(4)], D, rt0, nrt, TAIL_PAT)

    issue_wo(0, 10 * NCH * WO_TPC, 256)
    issue_w1(0, 8)
    _wait_all(wo_v, sems.at[S_WO])

    def wo_dot(m):
        lo = _mo(768 * m, 128)
        return _dot(o_s[:, pl.ds(lo, 768)], wo_v[pl.ds(lo, 768), :])

    def wo_a(ch, acc):
        issue_w1(8 + 2 * ch, 2)
        return acc + wo_dot(ch)
    att = loop(6, wo_a, jnp.zeros((1, D), f32))

    def wo_b(ch, acc):
        issue_w2a(6 * ch, 6)
        return acc + wo_dot(6 + ch)
    att = loop(2, wo_b, att)

    x1 = x + mod_s[:, 2 * D:3 * D] * att
    y_s[0:1, :] = _layernorm(x1) * (1.0 + mod_s[:, 4 * D:5 * D]) + mod_s[:, 3 * D:4 * D]
    y_s[1:2, :] = x1
    issue_w2a(12, 4)
    cp_b1.wait()
    b1 = b1_v[...].astype(f32)
    hh_s[...] = jnp.concatenate([b1[j:j + 1, :] for j in range(F // 128)], axis=1)
    _wait_all(w1_v, sems.at[S_W1])

    def w1_it(ch, carry):
        issue_w2a(16 + 4 * ch, 4)
        co = pl.multiple_of(ch * 384, 128)
        hh = hh_s[:, pl.ds(co, 384)] + _dot(y_s[0:1, :], w1_v[:, pl.ds(co, 384)])
        sp = jnp.log1p(jnp.exp(-jnp.abs(hh))) + jnp.maximum(hh, 0.0)
        hh_s[:, pl.ds(co, 384)] = hh * jnp.tanh(sp)
        return carry
    loop(4, w1_it)

    _issue_streams(w2_hbm, w2b_v, sems.at[S_W2 + 1], [(384 * m + 256, 128 * m) for m in range(2)], D, 0, 16, TAIL_PAT)
    for j in range(32):
        t, i = j // 2, j % 2
        part = sum(1 for e in range(1, len(CS)) if 8 * j >= sum(CS[:e]))
        _copy(w2_hbm, w2c_v, sems.at[S_W2 + 2 + part], 384 * (2 + i) + 256 + 8 * t, 8 * j, 8,
              0, 0, D, TAIL_PAT[j % len(TAIL_PAT)])
    for i in range(2):
        lo = 384 * (2 + i) + 256
        abt = jnp.broadcast_to(hh_s[:, lo:lo + 128], (128, 128)).T
        for t in range(16):
            ab_s[8 * (2 * t + i):8 * (2 * t + i) + 8, :] = abt[8 * t:8 * t + 8, :]

    _wait_all(w2a_v, sems.at[S_W2])
    act_a = jnp.concatenate([hh_s[:, 384 * m:384 * m + 256] for m in range(4)], axis=1)
    y_s[2:3, :] = _dot(act_a, w2a_v[...])
    _wait_all(w2b_v, sems.at[S_W2 + 1])
    act_b = jnp.concatenate([hh_s[:, 384 * m + 256:384 * m + 384] for m in range(2)], axis=1)
    gb = mod_s[:, 5 * D:6 * D]
    y_s[3:4, :] = y_s[1:2, :] + gb * (y_s[2:3, :] + _dot(act_b, w2b_v[...]))

    def vpu_part(r0, n, acc):
        for r in range(r0, r0 + n, 16):
            prod = w2c_v[r:r + 16, :].astype(f32) * jnp.concatenate([ab_s[r:r + 16, :]] * (D // 128), axis=1)
            pr = prod[0:8, :] + prod[8:16, :]
            acc = pr if acc is None else acc + pr
        return acc

    r0 = 0
    for e, n in enumerate(CS):
        _wait_all(w2c_v.at[pl.ds(r0, n), :], sems.at[S_W2 + 2 + e])
        acc = vpu_part(r0, n, None if e == 0 else y8_s[...])
        if e + 1 < len(CS):
            y8_s[...] = acc
        r0 += n
    o_ref[...] = (y_s[3:4, :] + gb * jnp.sum(acc, axis=0, keepdims=True)).astype(o_ref.dtype)


def _kernel(*refs):
    pl.run_scoped(functools.partial(_body, *refs), pltpu.SemaphoreType.DMA((NSEM,)))


@jax.jit
def pallas_adaLN_cond__sliding_block_cached__dense_activation_mish__decode_kernel(
    A_x: jax.Array,
    A_k_cache: jax.Array,
    A_v_cache: jax.Array,
    A_wq: jax.Array,
    A_wo: jax.Array,
    B_x: jax.Array,
    B_w1: jax.Array,
    B_b1: jax.Array,
    B_w2: jax.Array,
    c: jax.Array,
    w_mod: jax.Array,
):
    _, H, SK, dh = A_k_cache.shape
    W = min(4096, max(256, SK // 4))
    kt = jnp.swapaxes(A_k_cache, 2, 3).reshape(H * dh, SK)
    vt = jnp.swapaxes(A_v_cache, 2, 3).reshape(H * dh, SK)
    out = pl.pallas_call(
        _kernel,
        out_shape=jax.ShapeDtypeStruct((1, D), A_x.dtype),
        in_specs=[pl.BlockSpec(memory_space=pl.ANY)] * 10,
        out_specs=pl.BlockSpec(memory_space=pltpu.VMEM),
        scratch_shapes=[
            pltpu.VMEM((1, D), bf16), pltpu.VMEM((1, D), bf16), pltpu.VMEM((F // 128, 128), bf16),
            pltpu.VMEM((D, 6 * D), bf16), pltpu.VMEM((D, HQ * DH), bf16),
            pltpu.VMEM((2, R, W), bf16), pltpu.VMEM((2, R, W), bf16),
            pltpu.VMEM((HQ * DH, D), bf16), pltpu.VMEM((D, F), bf16),
            pltpu.VMEM((1024, D), bf16), pltpu.VMEM((256, D), bf16), pltpu.VMEM((256, D), bf16),
            pltpu.VMEM((1, 6 * D), f32), pltpu.VMEM((1, HQ * DH), f32), pltpu.VMEM((1, HQ * DH), f32),
            pltpu.VMEM((8, W), f32), pltpu.VMEM((8, W), f32), pltpu.VMEM((1, F), f32), pltpu.VMEM((8, D), f32),
            pltpu.VMEM((256, 128), f32), pltpu.VMEM((8, D), f32),
        ],
        compiler_params=pltpu.CompilerParams(vmem_limit_bytes=64 * 1024 * 1024, disable_bounds_checks=True),
    )(A_x.reshape(1, D), c, B_b1.reshape(F // 128, 128), w_mod, A_wq, kt, vt, A_wo, B_w1, B_w2)
    return out.reshape(A_x.shape)
```
